```python
import os as _os
_os.environ.setdefault("JAX_PLATFORMS", "cpu")
import jax
import jax.numpy as jnp

def _softmax(x, axis=-1):
    return jax.nn.softmax(x, axis=axis)
def _gelu(x):
    return jax.nn.gelu(x, approximate=True)
def _silu(x):
    return jax.nn.silu(x)
def _sigmoid(x):
    return jax.nn.sigmoid(x)
def _layernorm(x, axis=-1, eps=1e-5):
    m = jnp.mean(x, axis=axis, keepdims=True)
    v = jnp.var(x, axis=axis, keepdims=True)
    return (x - m) / jnp.sqrt(v + eps)
def _scatter_add(tgt, idx, src, axis=0):
    return tgt.at[idx].add(src)
def _segment_sum(src, seg, n):
    return jax.ops.segment_sum(src, seg, n)
class _Rng:
    def __init__(self, key):
        self._k = key
    def _next(self):
        self._k, sub = jax.random.split(self._k)
        return sub
    def normal(self, shape):
        return jax.random.normal(self._next(), shape, dtype=jnp.bfloat16)
    def randint(self, lo, hi, shape):
        return jax.random.randint(self._next(), shape, lo, hi, dtype=jnp.int32)
    def uniform(self, shape, lo=0.0, hi=1.0):
        return jax.random.uniform(self._next(), shape, jnp.bfloat16, lo, hi)
    def permutation(self, n):
        return jax.random.permutation(self._next(), n)


kernel_name = 'standalone__layernorm_linear__sampling'

def setup_inputs():
    _rng = _Rng(jax.random.key(int.from_bytes(__import__("os").urandom(4), "little")))
    _w = (lambda a: (lambda t: t.astype(jnp.bfloat16) if jnp.issubdtype(t.dtype, jnp.floating) else t)(jnp.asarray(a)))
    B, S, D = 1024, 32, 576
    return {
        "x": _w((lambda *s: _rng.normal(s) * 0.05)(B, S, D)),
        "g": _w((lambda *s: _rng.normal(s) * 0.05)(D) + 1.0),
        "b": _w((lambda *s: _rng.normal(s) * 0.05)(D)),
        "w": _w((lambda *s: _rng.normal(s) * 0.05)(D, D)),
    }

def reference(x, g, b, w):
    return (_layernorm(x, axis=-1) * g + b) @ w
```

```python
import jax
import jax.numpy as jnp
from jax import lax
import jax.experimental.pallas as pl
import jax.experimental.pallas.tpu as pltpu

EPS = 1e-5
f32 = jnp.float32
bf16 = jnp.bfloat16
u32 = jnp.uint32

S, D, B = 32, 576, 1024
KA = D + 16
CHUNK = 256
NTIES = 12
HEAD = (512, 512, 1024)
MID = 2
TAIL = (1024, 512, 512)


def _split3(v):
    h = v.astype(bf16).astype(f32)
    r = v - h
    m = r.astype(bf16).astype(f32)
    return h, m, r - m


def _prep_w(w_ref, g_ref, b_ref, wa_ref):
    wt = w_ref[...].astype(f32).T
    g = g_ref[...].astype(f32).reshape(1, D)
    b = b_ref[...].astype(f32).reshape(1, D)
    wg = (wt * g).astype(bf16)
    c = jnp.sum(wg.astype(f32), axis=1, keepdims=True)
    d = jnp.sum(wt * b, axis=1, keepdims=True)
    col = lax.broadcasted_iota(jnp.int32, (D, 16), 1)
    h, m, l = _split3(jnp.where(col < 6, c, d))
    ext = jnp.where((col == 2) | (col == 4) | (col == 8) | (col == 9), m,
                    jnp.where(col == 5, l, jnp.where(col < 10, h, 0.0)))
    wa = jnp.concatenate([wg, ext.astype(bf16)], axis=1)
    wa_ref[...] = pltpu.bitcast(wa, u32)


def _chunk(x_ref, o_ref, wa_ref, never, s, c0, T):
    rg = 8
    ng = D // rg
    per = ng // NTIES
    sh = x_ref[s, 0:rg, c0:c0 + T].astype(f32)
    sh = jnp.broadcast_to(sh[0:1, :], (rg, T))
    a1 = a2 = None
    col0 = []
    for i in range(ng):
        v = x_ref[s, i * rg:(i + 1) * rg, c0:c0 + T].astype(f32) - sh
        if a1 is None:
            a1, a2 = v, v * v
        else:
            a1 = a1 + v
            a2 = a2 + v * v
        if (i + 1) % per == 0:
            t = (i + 1) // per - 1
            w = wa_ref[8 * t:8 * t + 8, 0:128]
            for a in (a1, a2):
                ab = pltpu.bitcast(a, u32)
                for j in range(T // 128):
                    w = jnp.where(never, ab[:, j * 128:(j + 1) * 128], w)
            col0.append(w)
    col0.append(wa_ref[8 * NTIES:, 0:128])
    wa = jnp.concatenate([jnp.concatenate(col0, axis=0), wa_ref[:, 128:]], axis=1)
    wa = pltpu.bitcast(wa, bf16)
    s1 = jnp.sum(a1, axis=0, keepdims=True) * (1.0 / D)
    s2 = jnp.sum(a2, axis=0, keepdims=True) * (1.0 / D)
    var = jnp.maximum(s2 - s1 * s1, 0.0) + EPS
    r = lax.rsqrt(var)
    sd = var * r
    nm = -(sh[0:1, :] + s1)
    row = lax.broadcasted_iota(jnp.int32, (16, T), 0)
    h, m, l = _split3(jnp.where(row < 6, nm, sd))
    ext = jnp.where((row == 1) | (row == 4) | (row == 7) | (row == 9), m,
                    jnp.where(row == 3, l, jnp.where(row < 10, h, 0.0)))
    xa = jnp.concatenate([x_ref[s, :, c0:c0 + T], ext.astype(bf16)], axis=0)
    acc = jnp.dot(wa, xa, preferred_element_type=f32)
    o_ref[s, :, c0:c0 + T] = (acc * r).astype(bf16)


def _static_steps(lst, s0):
    out = []
    t = s0 * B
    for n in lst:
        s, c = divmod(t, B)
        out.append((s, n // B, 0, B) if n >= B else (s, 1, c, n))
        t += n
    return out


_NH = sum(HEAD) // B
_NT = sum(TAIL) // B
_NMID = (S - _NH - _NT) // MID
_HS = _static_steps(HEAD, 0)
_TS = _static_steps(TAIL, S - _NT)
_NSTEPS = len(_HS) + _NMID + len(_TS)


def _kernel(x_hbm, g_hbm, b_hbm, w_hbm, o_hbm, xbuf, obuf, wbuf, gbuf, bbuf, wa_ref, zref,
            isem, osem, psem):
    def desc(k):
        if k < len(_HS):
            return _HS[k]
        if k < len(_HS) + _NMID:
            return (_NH + (k - len(_HS)) * MID, MID, 0, B)
        return _TS[k - len(_HS) - _NMID]

    def in_cp(k, s, ns, c, n):
        return pltpu.make_async_copy(x_hbm.at[pl.ds(s, ns), :, pl.ds(c, n)],
                                     xbuf.at[pl.ds(s, ns), :, pl.ds(c, n)], isem.at[k])

    def out_cp(k, s, ns, c, n):
        return pltpu.make_async_copy(obuf.at[pl.ds(s, ns), :, pl.ds(c, n)],
                                     o_hbm.at[pl.ds(s, ns), :, pl.ds(c, n)], osem.at[k])

    def step(k, s, ns, c, n):
        in_cp(k, s, ns, c, n).wait()
        never = zref[...] != 0
        for j in range(ns):
            for c0 in range(c, c + n, CHUNK):
                _chunk(xbuf, obuf, wa_ref, never, s + j, c0, CHUNK)
        out_cp(k, s, ns, c, n).start()

    wcp = pltpu.make_async_copy(w_hbm, wbuf, psem.at[0])
    gcp = pltpu.make_async_copy(g_hbm, gbuf, psem.at[1])
    bcp = pltpu.make_async_copy(b_hbm, bbuf, psem.at[2])
    gcp.start()
    bcp.start()
    wcp.start()
    in_cp(0, *desc(0)).start()
    zref[...] = jnp.zeros(zref.shape, zref.dtype)
    wcp.wait()
    gcp.wait()
    bcp.wait()
    for k in range(1, _NSTEPS):
        in_cp(k, *desc(k)).start()
    _prep_w(wbuf, gbuf, bbuf, wa_ref)
    for k in range(len(_HS)):
        step(k, *desc(k))

    def body(i, carry):
        step(len(_HS) + i, _NH + i * MID, MID, 0, B)
        return carry

    lax.fori_loop(0, _NMID, body, 0)
    for k in range(len(_HS) + _NMID, _NSTEPS):
        step(k, *desc(k))
    for k in range(_NSTEPS):
        out_cp(k, *desc(k)).wait()


@jax.jit
def pallas_standalone__layernorm_linear__sampling_kernel(
    x: jax.Array,
    g: jax.Array,
    b: jax.Array,
    w: jax.Array,
):
    assert x.shape == (B, S, D)
    xt = jnp.transpose(x, (1, 2, 0))
    anyspec = pl.BlockSpec(memory_space=pl.ANY)
    out = pl.pallas_call(
        _kernel,
        in_specs=[anyspec] * 4,
        out_specs=anyspec,
        out_shape=jax.ShapeDtypeStruct((S, D, B), x.dtype),
        scratch_shapes=[
            pltpu.VMEM((S, D, B), bf16), pltpu.VMEM((S, D, B), bf16),
            pltpu.VMEM((D, D), bf16), pltpu.VMEM((D,), bf16), pltpu.VMEM((D,), bf16),
            pltpu.VMEM((D // 2, KA), u32), pltpu.VMEM((8, 128), jnp.int32),
            pltpu.SemaphoreType.DMA((_NSTEPS,)), pltpu.SemaphoreType.DMA((_NSTEPS,)),
            pltpu.SemaphoreType.DMA((3,)),
        ],
        compiler_params=pltpu.CompilerParams(vmem_limit_bytes=110 * 1024 * 1024),
    )(xt, g, b, w)
    return jnp.transpose(out, (2, 0, 1))
```

```python
import jax
import jax.numpy as jnp
from jax import lax
import jax.experimental.pallas as pl
import jax.experimental.pallas.tpu as pltpu

EPS = 1e-5
f32 = jnp.float32
bf16 = jnp.bfloat16
u32 = jnp.uint32

S, D, B = 32, 576, 1024
H = D // 2
KH = 256
KR = D - 2 * KH + 16
T = 256
CPS = B // T
NCH = S * CPS

HEAD = (2, 4, 10)
MID = 16
OUTP = (4, 4, 4, 2, 1, 1)
TIE_SPAN = 48
ORDER = (1, 4, 0, 3, 6, 2, 'r0', 5, 'r1')


def _prep_w(w_ref, g_ref, b_ref, la_ref, lr_ref):
    wt = w_ref[...].astype(f32).T
    g = g_ref[...].astype(f32).reshape(1, D)
    b = b_ref[...].astype(f32).reshape(1, D)
    a = wt * g
    d = jnp.sum(wt * b, axis=1, keepdims=True)
    a11, a12 = a[:H, :KH], a[:H, KH:2 * KH]
    a21, a22 = a[H:, :KH], a[H:, KH:2 * KH]
    ls = (a11 + a22, a21 + a22, a11, a22, a11 + a12, a21 - a11, a12 - a22)
    for i, l in enumerate(ls):
        la_ref[i] = pltpu.bitcast(l.astype(bf16), u32)
    col = lax.broadcasted_iota(jnp.int32, (D, 16), 1)
    dh = d.astype(bf16).astype(f32)
    ext = jnp.where(col == 0, dh, jnp.where(col == 1, d - dh, 0.0))
    lr = jnp.concatenate([a[:, 2 * KH:], ext], axis=1).astype(bf16)
    lr_ref[...] = pltpu.bitcast(lr, u32)


def _stats(x_ref, s, c0, ties):
    rg = 8
    ng = D // rg
    sh = x_ref[s, 0:rg, pl.ds(c0, T)].astype(f32)
    sh = jnp.broadcast_to(sh[0:1, :], (rg, T))
    a1 = a2 = None
    for i in range(ng):
        v = x_ref[s, i * rg:(i + 1) * rg, pl.ds(c0, T)].astype(f32) - sh
        if a1 is None:
            a1, a2 = v, v * v
        else:
            a1 = a1 + v
            a2 = a2 + v * v
        if ties is not None:
            t = ((i + 1) * TIE_SPAN) // ng - 1
            tn = ((i + 2) * TIE_SPAN) // ng - 1
            if (tn != t or i == ng - 1) and t >= 0:
                for a in (a1, a2):
                    ab = pltpu.bitcast(a, u32)
                    ties.setdefault(t, []).extend([ab[:, :128], ab[:, 128:]])
    s1 = jnp.sum(a1, axis=0, keepdims=True) * (1.0 / D)
    s2 = jnp.sum(a2, axis=0, keepdims=True) * (1.0 / D)
    var = jnp.maximum(s2 - s1 * s1, 0.0) + EPS
    r = jnp.broadcast_to(lax.rsqrt(var), (8, T))
    return sh + s1, r


def _matmuls(la_ref, lr_ref, x_ref, zs, mr, o_ref, s, c0, ties, never, top_done=None):
    m, r = mr[0][0:1], mr[1][0:1]
    m1, m2, r1, r2 = m[:, :128], m[:, 128:], r[:, :128], r[:, 128:]
    mu = m1 * r1 + m2 * r2

    def q(z, kh, tb):
        v = x_ref[s + zs[z], kh * KH:(kh + 1) * KH, pl.ds(c0, T)].astype(f32)
        return v[:, tb * 128:(tb + 1) * 128]

    def rhs(i):
        if i == 0:
            v = q(i, 0, 0) * r1 + q(i, 1, 1) * r2 - mu
        elif i == 1:
            v = (q(i, 0, 0) - m1) * r1
        elif i == 2:
            v = (q(i, 0, 1) - q(i, 1, 1)) * r2
        elif i == 3:
            v = (q(i, 1, 0) - q(i, 0, 0)) * r1
        elif i == 4:
            v = (q(i, 1, 1) - m2) * r2
        elif i == 5:
            v = q(i, 0, 0) * r1 + q(i, 0, 1) * r2 - mu
        else:
            v = q(i, 1, 0) * r1 + q(i, 1, 1) * r2 - mu
        return v.astype(bf16)

    def tied(i, d):
        col0 = []
        for j in range(H // 16):
            w = la_ref[i, 8 * j:8 * j + 8, 0:128]
            for tv in ties.get((H // 16) * (d // 2) + j, []):
                w = jnp.where(never, tv, w)
            col0.append(w)
        return jnp.concatenate([jnp.concatenate(col0, axis=0), la_ref[i, :, 128:]], axis=1)

    row = lax.broadcasted_iota(jnp.int32, (16, T), 0)
    res = {}
    for d, i in enumerate(ORDER):
        if isinstance(i, str):
            h = int(i[1])
            l = lr_ref[h * (H // 2):(h + 1) * (H // 2), :]
            xr = (x_ref[s + zs[7 + h], 2 * KH:, pl.ds(c0, T)].astype(f32) - m) * r
            rh = jnp.concatenate([xr, jnp.where(row < 2, 1.0, 0.0)], axis=0).astype(bf16)
        else:
            l = tied(i, d) if d % 2 == 0 else la_ref[i]
            rh = rhs(i)
        res[i] = jnp.dot(pltpu.bitcast(l, bf16), rh, preferred_element_type=f32)
        if i == 'r0':
            c11 = res[0] + res[3] - res[4] + res[6]
            top = jnp.concatenate([c11, res[2] + res[4]], axis=1) + res['r0']
            o_ref[s, 0:H, pl.ds(c0, T)] = top.astype(bf16)
            if top_done is not None:
                top_done()
    c22 = res[0] - res[1] + res[2] + res[5]
    bot = jnp.concatenate([res[1] + res[3], c22], axis=1) + res['r1']
    o_ref[s, H:, pl.ds(c0, T)] = bot.astype(bf16)


def _rects(a, b):
    out = []
    while a < b:
        s, c = divmod(a, CPS)
        if c == 0 and b - a >= CPS:
            n = (b - a) // CPS
            out.append((s, n, 0, B))
            a += n * CPS
        else:
            e = min(b, (s + 1) * CPS)
            out.append((s, 1, c * T, (e - a) * T))
            a = e
    return out


_NH = sum(HEAD)
_NMID = (NCH - _NH) // MID
_MSL = MID // CPS
_HB = [sum(HEAD[:k]) for k in range(len(HEAD) + 1)]
_IN_PIECES = [_rects(0, 1)] + [_rects(_HB[k] + 1, _HB[k + 1] + 1) for k in range(len(HEAD))]
_LP = _rects(1, MID + 1)
_NSEM_IN = sum(len(p) for p in _IN_PIECES) + _NMID * len(_LP)
assert _NH + _NMID * MID == NCH and sum(OUTP) == MID and _NH % CPS == 0 and MID % CPS == 0
assert TIE_SPAN <= 3 * (H // 16) and OUTP[-1] == 1


def _kernel(x_hbm, g_hbm, b_hbm, w_hbm, o_hbm, xbuf, obuf, wbuf, gbuf, bbuf, la_ref, lr_ref,
            zref, zs_ref, isem, osem, psem):
    def in_cp(k, s, ns, c, n):
        return pltpu.make_async_copy(x_hbm.at[pl.ds(s, ns), :, pl.ds(c, n)],
                                     xbuf.at[pl.ds(s, ns), :, pl.ds(c, n)], isem.at[k])

    def out_start(s, ns, c, n, r0=0, nr=D):
        pltpu.make_async_copy(obuf.at[pl.ds(s, ns), pl.ds(r0, nr), pl.ds(c, n)],
                              o_hbm.at[pl.ds(s, ns), pl.ds(r0, nr), pl.ds(c, n)],
                              osem.at[0]).start(priority=1)

    static_in = []
    base = 0
    for p in _IN_PIECES:
        static_in.append([in_cp(base + j, *rc) for j, rc in enumerate(p)])
        base += len(p)

    def loop_in(i, j):
        s, ns, c, n = _LP[j]
        return in_cp(base + i * len(_LP) + j, _NH // CPS + i * _MSL + s, ns, c, n)

    def run(chunks, nxt, mr, after=None):
        never = zref[...] != 0
        zs = [zs_ref[i] for i in range(9)]
        for ci, (ss, c0) in enumerate(chunks):
            ties = {}
            nx = chunks[ci + 1] if ci + 1 < len(chunks) else nxt
            nmr = _stats(xbuf, *nx, ties)
            top_done = None
            if after is not None and ci == len(chunks) - 1:
                top_done = lambda: out_start(ss, 1, c0, T, 0, H)
            _matmuls(la_ref, lr_ref, xbuf, zs, mr, obuf, ss, c0, ties, never, top_done)
            mr = nmr
            if after is not None:
                after(ci)
        return mr

    wcp = pltpu.make_async_copy(w_hbm, wbuf, psem.at[0])
    gcp = pltpu.make_async_copy(g_hbm, gbuf, psem.at[1])
    bcp = pltpu.make_async_copy(b_hbm, bbuf, psem.at[2])
    gcp.start()
    bcp.start()
    wcp.start()
    for p in static_in:
        for c in p:
            c.start(priority=1)
    for i in range(_NMID):
        for j in range(len(_LP) - (1 if i == _NMID - 1 else 0)):
            loop_in(i, j).start(priority=1)
    zref[...] = jnp.zeros(zref.shape, zref.dtype)
    for i in range(9):
        zs_ref[i] = 0
    wcp.wait()
    gcp.wait()
    bcp.wait()
    _prep_w(wbuf, gbuf, bbuf, la_ref, lr_ref)
    for c in static_in[0]:
        c.wait()
    mr = _stats(xbuf, 0, 0, None)

    def ch(a):
        return a // CPS, (a % CPS) * T

    for k in range(len(HEAD)):
        for c in static_in[k + 1]:
            c.wait()
        mr = run([ch(a) for a in range(_HB[k], _HB[k + 1])], ch(_HB[k + 1]), mr)
    out_start(0, _NH // CPS, 0, B)

    ends = {}
    t = 0
    for n in OUTP:
        ends[t + n - 1] = (t, t + n)
        t += n

    def body(i, mr):
        s = _NH // CPS + i * _MSL
        for j in range(len(_LP) - 1):
            loop_in(i, j).wait()
        pl.when(i + 1 < _NMID)(lambda: loop_in(i, len(_LP) - 1).wait())

        def after(ci):
            for (ds, ns, c, n) in _rects(*ends.get(ci, (0, 0))):
                if ci == MID - 1:
                    out_start(s + ds, ns, c, n, H, H)
                else:
                    out_start(s + ds, ns, c, n)

        chunks = [(s + a // CPS, (a % CPS) * T) for a in range(MID)]
        return run(chunks, (jnp.minimum(s + _MSL, S - 1), 0), mr, after)

    lax.fori_loop(0, _NMID, body, mr)
    pltpu.make_async_copy(obuf, o_hbm, osem.at[0]).wait()


@jax.jit
def pallas_standalone__layernorm_linear__sampling_kernel(
    x: jax.Array,
    g: jax.Array,
    b: jax.Array,
    w: jax.Array,
):
    assert x.shape == (B, S, D)
    xt = jnp.transpose(x, (1, 2, 0))
    anyspec = pl.BlockSpec(memory_space=pl.ANY)
    out = pl.pallas_call(
        _kernel,
        in_specs=[anyspec] * 4,
        out_specs=anyspec,
        out_shape=jax.ShapeDtypeStruct((S, D, B), x.dtype),
        scratch_shapes=[
            pltpu.VMEM((S, D, B), bf16), pltpu.VMEM((S, D, B), bf16),
            pltpu.VMEM((D, D), bf16), pltpu.VMEM((D,), bf16), pltpu.VMEM((D,), bf16),
            pltpu.VMEM((7, H // 2, KH), u32), pltpu.VMEM((D // 2, KR), u32),
            pltpu.VMEM((8, 128), jnp.int32), pltpu.SMEM((16,), jnp.int32),
            pltpu.SemaphoreType.DMA((_NSEM_IN,)), pltpu.SemaphoreType.DMA((1,)),
            pltpu.SemaphoreType.DMA((3,)),
        ],
        compiler_params=pltpu.CompilerParams(
            vmem_limit_bytes=110 * 1024 * 1024,
            disable_bounds_checks=True,
            disable_semaphore_checks=True,
        ),
    )(xt, g, b, w)
    return jnp.transpose(out, (2, 0, 1))
```

```python
import jax
import jax.numpy as jnp
from jax import lax
import jax.experimental.pallas as pl
import jax.experimental.pallas.tpu as pltpu

EPS = 1e-5
f32 = jnp.float32
bf16 = jnp.bfloat16
u32 = jnp.uint32

S, D, B = 32, 576, 1024
H = D // 2
Q = D // 4
KH = 256
KR = D - 2 * KH + 16
T = 256
T2 = 2 * T
CPS = B // T
NCH = S * CPS

HEAD = (2, 6, 8)
MID = 16
ORDER = (4, 3, 0, 2, 6, 1, 5)
INNER = (1, 4, 0, 3, 6, 2, 5)
FLIP = (6, 4, 5, 1)
TOP_AFTER = 9
TIE_SPAN = 99
KICK_ROUND = 3
HOLD = (2, 3, 4)
BAND = 24
NZ = 4
ZOF = {0: 1, 5: 2, 6: 2, 2: 3, 3: 3, 1: 0, 4: 0}


def _lhs_combos(a11, a12, a21, a22):
    return [a11 + a22, a21 + a22, a11, a22, a11 + a12, a21 - a11, a12 - a22]


def _out_combos(p):
    return (p(0) + p(3) - p(4) + p(6), p(2) + p(4), p(1) + p(3), p(0) - p(1) + p(2) + p(5))


def _rounds():
    a, b = ORDER[0], ORDER[1]
    st = [(a, 1), (a, 4), (b, 1), (b, 4)] + [(a, j) for j in INNER[2:]] + [(b, j) for j in INNER[2:]]
    st += [(i, j) for i in ORDER[2:] for j in INNER]
    rs = []
    for k in range((len(st) + 3) // 4):
        rs.append(st[4 * k:4 * k + 4])
        if k + 1 == TOP_AFTER:
            rs.append(['r0'])
    rs.append(['r1'])
    return rs


_ROUNDS = _rounds()


def _prep_w(w_ref, g_ref, b_ref, lb_ref, lr_ref):
    g = g_ref[...].astype(f32).reshape(1, D)
    b = b_ref[...].astype(f32).reshape(1, D)
    rowi = lax.broadcasted_iota(jnp.int32, (16, D), 0)
    d = jnp.dot(jnp.broadcast_to(b, (16, D)).astype(bf16), w_ref[...],
                preferred_element_type=f32)
    dh = d.astype(bf16).astype(f32)
    dd = jnp.where(rowi == 0, dh, jnp.where(rowi == 1, d - dh, 0.0)).astype(bf16)
    a = w_ref[0:2 * KH, :].astype(f32).T * g[:, :2 * KH]
    gr = jnp.concatenate([g[:, 2 * KH:], jnp.ones((1, 16), f32)], axis=1)
    ar = jnp.concatenate([w_ref[2 * KH:, :], dd], axis=0).astype(f32).T * gr
    c = jnp.sum(a[:, :128], axis=1, keepdims=True) * (1.0 / 128)
    a = a - c
    lane = lax.broadcasted_iota(jnp.int32, (1, KR), 1)
    ar = jnp.where(lane < D - 2 * KH, ar - c, ar)
    lr_ref[...] = pltpu.bitcast(ar.astype(bf16), u32)
    for i, l in enumerate(_lhs_combos(a[:H, :KH], a[:H, KH:], a[H:, :KH], a[H:, KH:])):
        for j, ll in enumerate(_lhs_combos(l[:Q, :128], l[:Q, 128:], l[Q:, :128], l[Q:, 128:])):
            lb_ref[7 * i + j] = pltpu.bitcast(ll.astype(bf16), u32)


def _stats(x_ref, s, c0, ties):
    rg = 8
    ng = D // rg
    sh = x_ref[s, 0:rg, pl.ds(c0, T2)].astype(f32)
    sh = jnp.broadcast_to(sh[0:1, :], (rg, T2))
    a1 = a2 = None
    for i in range(ng):
        v = x_ref[s, i * rg:(i + 1) * rg, pl.ds(c0, T2)].astype(f32) - sh
        if a1 is None:
            a1, a2 = v, v * v
        else:
            a1 = a1 + v
            a2 = a2 + v * v
        if ties is not None:
            j = (1, 3)[i % 2]
            ties[((i + 1) * TIE_SPAN) // ng - 1] = pltpu.bitcast(a2, u32)[:, j * 128:(j + 1) * 128]
    s1 = jnp.sum(a1, axis=0, keepdims=True) * (1.0 / D)
    s2 = jnp.sum(a2, axis=0, keepdims=True) * (1.0 / D)
    var = jnp.maximum(s2 - s1 * s1, 0.0) + EPS
    r = jnp.broadcast_to(lax.rsqrt(var), (8, T2))
    return sh + s1, r


def _block(acc_ref, lb_ref, lr_ref, x_ref, zs, mr, o_ref, s, c0, ties, never, done, kick):
    m, r = mr[0][0:1], mr[1][0:1]
    m_u, m_v, r_u, r_v = m[:, :T], m[:, T:], r[:, :T], r[:, T:]
    mu = m_u * r_u + m_v * r_v

    def hv(v, t):
        return v[:, t * 128:(t + 1) * 128]

    def operand(i, kh, t):
        def q(kk, uv):
            k0 = kk * KH + kh * 128
            v = x_ref[s + zs[ZOF[i]], k0:k0 + 128, pl.ds(c0 + uv * T, T)]
            return hv(v.astype(f32), t)
        if i == 0:
            return q(0, 0) * hv(r_u, t) + q(1, 1) * hv(r_v, t) - hv(mu, t)
        if i == 1:
            return (q(0, 0) - hv(m_u, t)) * hv(r_u, t)
        if i == 2:
            return (q(0, 1) - q(1, 1)) * hv(r_v, t)
        if i == 3:
            return (q(1, 0) - q(0, 0)) * hv(r_u, t)
        if i == 4:
            return (q(1, 1) - hv(m_v, t)) * hv(r_v, t)
        if i == 5:
            return q(0, 0) * hv(r_u, t) + q(0, 1) * hv(r_v, t) - hv(mu, t)
        return q(1, 0) * hv(r_u, t) + q(1, 1) * hv(r_v, t) - hv(mu, t)

    def tied(ref2d, base):
        w_ = ref2d.shape[1]
        rows = []
        for j in range(ref2d.shape[0] // 8):
            w = ref2d[8 * j:8 * j + 8, :]
            if base + j in ties:
                w = jnp.where(never[:, :w_], ties[base + j][:, :w_], w)
            rows.append(w)
        return jnp.concatenate(rows, axis=0)

    res, ops, lvl1 = {}, {}, {}
    rest = None
    te = 0
    for ri, rnd in enumerate(_ROUNDS):
        for pos, item in enumerate(rnd):
            if isinstance(item, str):
                h = int(item[1])
                ref2d = lr_ref.at[h * Q:(h + 1) * Q, :]
                if rest is None:
                    xr = (x_ref[s + zs[0], 2 * KH:, pl.ds(c0, T2)].astype(f32) - m) * r
                    row = lax.broadcasted_iota(jnp.int32, (16, T2), 0)
                    rest = jnp.concatenate([xr, jnp.where(row < 2, 1.0, 0.0)], axis=0).astype(bf16)
                rh = rest
            else:
                i, j = item
                if i not in ops:
                    ops[i] = [[operand(i, kh, 1 - t if i in FLIP else t) for t in range(2)]
                              for kh in range(2)]
                (b11, b12), (b21, b22) = ops[i]
                rh = (lambda: b11 + b22, lambda: b11, lambda: b12 - b22, lambda: b21 - b11,
                      lambda: b22, lambda: b11 + b12, lambda: b21 + b22)[j]().astype(bf16)
                ref2d = lb_ref.at[7 * i + j]
            if pos == 0:
                l = tied(ref2d, te)
                te += ref2d.shape[0] // 8
            else:
                l = ref2d[...]
                if pos == 1 and ri == KICK_ROUND and kick is not None:
                    l = jnp.concatenate([jnp.where(never, kick, l[:8]), l[8:]], axis=0)
            res[item] = jnp.dot(pltpu.bitcast(l, bf16), rh, preferred_element_type=f32)
            if item == 'r0':
                top = jnp.concatenate([lvl1[0] + lvl1[3] - lvl1[4] + lvl1[6], lvl1[2] + lvl1[4]],
                                      axis=1) + res['r0']
                o_ref[s, 0:H, pl.ds(c0, T2)] = top.astype(bf16)
                if done is not None:
                    done(0, H)
            elif item != 'r1' and all((item[0], j) in res for j in range(7)):
                i = item[0]
                c11, c12, c21, c22 = _out_combos(lambda j: res[(i, j)])
                if i in FLIP:
                    c11, c12, c21, c22 = c12, c11, c22, c21
                v = jnp.concatenate([jnp.concatenate([c11, c12], axis=1),
                                     jnp.concatenate([c21, c22], axis=1)], axis=0)
                if i != ORDER[-1]:
                    acc_ref[ORDER.index(i)] = v
                    v = acc_ref[ORDER.index(i)]
                lvl1[i] = v
    bot = jnp.concatenate([lvl1[1] + lvl1[3], lvl1[0] - lvl1[1] + lvl1[2] + lvl1[5]], axis=1)
    bot = (bot + res['r1']).astype(bf16)
    if done is None:
        o_ref[s, H:, pl.ds(c0, T2)] = bot
    else:
        o_ref[s, H:H + Q, pl.ds(c0, T2)] = bot[:Q]
        done(H, Q)
        o_ref[s, H + Q:, pl.ds(c0, T2)] = bot[Q:]
        done(H + Q, Q)


def _rects(a, b):
    out = []
    while a < b:
        s, c = divmod(a, CPS)
        if c == 0 and b - a >= CPS:
            n = (b - a) // CPS
            out.append((s, n, 0, B))
            a += n * CPS
        else:
            e = min(b, (s + 1) * CPS)
            out.append((s, 1, c * T, (e - a) * T))
            a = e
    return out


_NH = sum(HEAD)
_NMID = (NCH - _NH) // MID
_MSL = MID // CPS
_HB = [sum(HEAD[:k]) for k in range(len(HEAD) + 1)]
_IN_PIECES = [_rects(0, 2)] + [_rects(_HB[k] + 2, _HB[k + 1] + 2) for k in range(len(HEAD))]
_LP = _rects(2, MID + 2)
_NSEM_IN = sum(len(p) for p in _IN_PIECES) + _NMID * len(_LP)
assert _NH + _NMID * MID == NCH and _NH % CPS == 0 and MID % CPS == 0


def _kernel(x_hbm, g_hbm, b_hbm, w_hbm, o_hbm, xbuf, obuf, wbuf, gbuf, bbuf, lb_ref, lr_ref,
            acc_ref, zref, zs_ref, isem, osem, psem):
    def in_cp(k, s, ns, c, n):
        return pltpu.make_async_copy(x_hbm.at[pl.ds(s, ns), :, pl.ds(c, n)],
                                     xbuf.at[pl.ds(s, ns), :, pl.ds(c, n)], isem.at[k])

    def out1(s, ns, c, n, r0, nr):
        pltpu.make_async_copy(obuf.at[pl.ds(s, ns), pl.ds(r0, nr), pl.ds(c, n)],
                              o_hbm.at[pl.ds(s, ns), pl.ds(r0, nr), pl.ds(c, n)],
                              osem.at[0]).start(priority=1)

    def out_start(s, c, n, r0=0, nr=D):
        for cc in range(0, n, 128):
            out1(s, 1, c + cc, 128, r0, nr)

    static_in = []
    base = 0
    for p in _IN_PIECES:
        static_in.append([in_cp(base + j, *rc) for j, rc in enumerate(p)])
        base += len(p)

    def loop_in(i, j):
        s, ns, c, n = _LP[j]
        return in_cp(base + i * len(_LP) + j, _NH // CPS + i * _MSL + s, ns, c, n)

    def run(blocks, nxt, mr, zs, after=None, last_done=None):
        never = zref[...] != 0
        kick = None
        for bi, (ss, c0) in enumerate(blocks):
            ties = {}
            nx = blocks[bi + 1] if bi + 1 < len(blocks) else nxt
            nmr = _stats(xbuf, *nx, ties)
            done = None
            if last_done is not None and bi == len(blocks) - 1:
                done = lambda r0, nr: last_done(ss, c0, r0, nr)
            _block(acc_ref.at[bi % 2], lb_ref, lr_ref, xbuf, zs, mr, obuf, ss, c0, ties, never,
                   done, kick)
            mr = nmr
            kick = after(bi) if after is not None else None
        return mr

    wcp = pltpu.make_async_copy(w_hbm, wbuf, psem.at[0])
    gcp = pltpu.make_async_copy(g_hbm, gbuf, psem.at[1])
    bcp = pltpu.make_async_copy(b_hbm, bbuf, psem.at[2])
    gcp.start()
    bcp.start()
    wcp.start()
    for p in static_in:
        for c in p:
            c.start(priority=1)
    for i in range(_NMID):
        for j in range(len(_LP) - (1 if i == _NMID - 1 else 0)):
            loop_in(i, j).start(priority=1)
    zref[...] = jnp.zeros(zref.shape, zref.dtype)
    for i in range(NZ):
        zs_ref[i] = 0
    wcp.wait()
    gcp.wait()
    bcp.wait()
    _prep_w(wbuf, gbuf, bbuf, lb_ref, lr_ref)
    for c in static_in[0]:
        c.wait()
    mr = _stats(xbuf, 0, 0, None)

    def ch(a):
        return a // CPS, (a % CPS) * T

    for k in range(len(HEAD)):
        zs = [zs_ref[i] for i in range(NZ)]
        for c in static_in[k + 1]:
            c.wait()
        mr = run([ch(a) for a in range(_HB[k], _HB[k + 1], 2)], ch(_HB[k + 1]), mr, zs)

    nblk = MID // 2
    hi, hb, ng = HOLD
    nbl = (hb + 1) // 2
    nb = _NH // CPS + hi * _MSL + nbl
    bands = list(range(0, D, BAND))
    per = len(bands) // ng

    def body(i, mr):
        s = _NH // CPS + i * _MSL
        zs = [zs_ref[j] for j in range(NZ)]
        for j in range(len(_LP) - 1):
            loop_in(i, j).wait()
        pl.when(i + 1 < _NMID)(lambda: loop_in(i, len(_LP) - 1).wait())

        def guarded(slab, fn):
            pl.when(i >= (hi if slab >= nbl else hi + 1))(fn)

        def after(bi):
            started = False
            if hb <= bi < hb + ng:
                @pl.when(i == hi)
                def _():
                    for rr in bands[(bi - hb) * per:(bi - hb + 1) * per]:
                        out1(0, nb, 0, B, rr, BAND)
                started = True
            if bi == nblk - 2:
                guarded(bi // 2, lambda: out_start(s + bi // 2, 0, T2))
                started = True
            elif bi % 2 == 1 and bi < nblk - 1:
                guarded(bi // 2, lambda: out_start(s + bi // 2, 0, B))
                started = True
            if not started or bi + 1 == nblk:
                return None
            ns, nc = s + (bi + 1) // 2, ((bi + 1) % 2) * T2
            obuf[ns, 0:8, pl.ds(nc, T)] = jnp.zeros((8, T), bf16)
            return pltpu.bitcast(obuf[ns, 0:8, pl.ds(nc, T)].astype(f32)[:, :128], u32)

        def last_done(ss, c0, r0, nr):
            guarded(_MSL - 1, lambda: out_start(ss, c0, T2, r0, nr))

        blocks = [(s + bi // 2, (bi % 2) * T2) for bi in range(nblk)]
        return run(blocks, (jnp.minimum(s + _MSL, S - 1), 0), mr, zs, after, last_done)

    lax.fori_loop(0, _NMID, body, mr)
    pltpu.make_async_copy(obuf, o_hbm, osem.at[0]).wait()


@jax.jit
def pallas_standalone__layernorm_linear__sampling_kernel(
    x: jax.Array,
    g: jax.Array,
    b: jax.Array,
    w: jax.Array,
):
    assert x.shape == (B, S, D)
    xt = jnp.transpose(x, (1, 2, 0))
    anyspec = pl.BlockSpec(memory_space=pl.ANY)
    out = pl.pallas_call(
        _kernel,
        in_specs=[anyspec] * 4,
        out_specs=anyspec,
        out_shape=jax.ShapeDtypeStruct((S, D, B), x.dtype),
        scratch_shapes=[
            pltpu.VMEM((S, D, B), bf16), pltpu.VMEM((S, D, B), bf16),
            pltpu.VMEM((D, D), bf16), pltpu.VMEM((D,), bf16), pltpu.VMEM((D,), bf16),
            pltpu.VMEM((49, Q // 2, 128), u32), pltpu.VMEM((D // 2, KR), u32),
            pltpu.VMEM((2, 6, H, T), f32),
            pltpu.VMEM((8, 128), jnp.int32), pltpu.SMEM((NZ,), jnp.int32),
            pltpu.SemaphoreType.DMA((_NSEM_IN,)), pltpu.SemaphoreType.DMA((1,)),
            pltpu.SemaphoreType.DMA((3,)),
        ],
        compiler_params=pltpu.CompilerParams(
            vmem_limit_bytes=110 * 1024 * 1024,
            disable_bounds_checks=True,
            disable_semaphore_checks=True,
        ),
    )(xt, g, b, w)
    return jnp.transpose(out, (2, 0, 1))
```

```python
import jax
import jax.numpy as jnp
from jax import lax
import jax.experimental.pallas as pl
import jax.experimental.pallas.tpu as pltpu

EPS = 1e-5
f32 = jnp.float32
bf16 = jnp.bfloat16
u32 = jnp.uint32

S, D, B = 32, 576, 1024
H = D // 2
Q = D // 4
KH = 256
KR = D - 2 * KH + 16
T = 256
T2 = 2 * T
CPS = B // T
NCH = S * CPS

HEAD = (2, 4, 2, 8)
MID = 16
ORDER = (4, 1, 2, 3, 0, 6, 5)
INNER = (1, 4, 0, 3, 6, 2, 5)
FLIP = (6, 4, 5, 1)
TOP_AFTER = 11
TIE_SPAN = 108
KICK_ROUND = 3
HOLD = (2, 3, 4)
BAND = 24
NZ = 4
ZOF = {0: 1, 5: 2, 6: 2, 2: 3, 3: 3, 1: 0, 4: 0}


def _lhs_combos(a11, a12, a21, a22):
    return [a11 + a22, a21 + a22, a11, a22, a11 + a12, a21 - a11, a12 - a22]


def _out_combos(p):
    return (p(0) + p(3) - p(4) + p(6), p(2) + p(4), p(1) + p(3), p(0) - p(1) + p(2) + p(5))


def _rounds():
    a, b = ORDER[0], ORDER[1]
    st = [(a, 1), (a, 4), (b, 1), (b, 4)] + [(a, j) for j in INNER[2:]] + [(b, j) for j in INNER[2:]]
    st += [(i, j) for i in ORDER[2:] for j in INNER]
    rs = []
    for k in range((len(st) + 3) // 4):
        rs.append(st[4 * k:4 * k + 4])
        if k + 1 == TOP_AFTER:
            rs.append(['r0'])
    rs.append(['r1'])
    return rs


_ROUNDS = _rounds()


def _prep_w(w_ref, g_ref, b_ref, lb_ref, lr_ref):
    g = g_ref[...].astype(f32).reshape(1, D)
    b = b_ref[...].astype(f32).reshape(1, D)
    rowi = lax.broadcasted_iota(jnp.int32, (16, D), 0)
    d = jnp.dot(jnp.broadcast_to(b, (16, D)).astype(bf16), w_ref[...],
                preferred_element_type=f32)
    dh = d.astype(bf16).astype(f32)
    dd = jnp.where(rowi == 0, dh, jnp.where(rowi == 1, d - dh, 0.0)).astype(bf16)
    a = w_ref[0:2 * KH, :].astype(f32).T * g[:, :2 * KH]
    gr = jnp.concatenate([g[:, 2 * KH:], jnp.ones((1, 16), f32)], axis=1)
    ar = jnp.concatenate([w_ref[2 * KH:, :], dd], axis=0).astype(f32).T * gr
    c = jnp.sum(a[:, :128], axis=1, keepdims=True) * (1.0 / 128)
    a = a - c
    lane = lax.broadcasted_iota(jnp.int32, (1, KR), 1)
    ar = jnp.where(lane < D - 2 * KH, ar - c, ar)
    lr_ref[...] = pltpu.bitcast(ar.astype(bf16), u32)
    for i, l in enumerate(_lhs_combos(a[:H, :KH], a[:H, KH:], a[H:, :KH], a[H:, KH:])):
        for j, ll in enumerate(_lhs_combos(l[:Q, :128], l[:Q, 128:], l[Q:, :128], l[Q:, 128:])):
            lb_ref[7 * i + j] = pltpu.bitcast(ll.astype(bf16), u32)


def _stats(x_ref, s, c0, ties):
    rg = 8
    ng = D // rg
    sh = x_ref[s, 0:rg, pl.ds(c0, T2)].astype(f32)
    sh = jnp.broadcast_to(sh[0:1, :], (rg, T2))
    a1 = a2 = None
    for i in range(ng):
        v = x_ref[s, i * rg:(i + 1) * rg, pl.ds(c0, T2)].astype(f32) - sh
        if a1 is None:
            a1, a2 = v, v * v
        else:
            a1 = a1 + v
            a2 = a2 + v * v
        if ties is not None:
            j = (1, 3)[i % 2]
            ties[((i + 1) * TIE_SPAN) // ng - 1] = pltpu.bitcast(a2, u32)[:, j * 128:(j + 1) * 128]
    s1 = jnp.sum(a1, axis=0, keepdims=True) * (1.0 / D)
    s2 = jnp.sum(a2, axis=0, keepdims=True) * (1.0 / D)
    var = jnp.maximum(s2 - s1 * s1, 0.0) + EPS
    r = jnp.broadcast_to(lax.rsqrt(var), (8, T2))
    return sh + s1, r


def _block(acc_ref, lb_ref, lr_ref, x_ref, zs, mr, o_ref, s, c0, ties, never, done, kick,
           balance):
    m, r = mr[0][0:1], mr[1][0:1]
    m_u, m_v, r_u, r_v = m[:, :T], m[:, T:], r[:, :T], r[:, T:]
    mu = m_u * r_u + m_v * r_v

    def hv(v, t):
        return v[:, t * 128:(t + 1) * 128]

    def operand(i, kh, t):
        def q(kk, uv):
            k0 = kk * KH + kh * 128
            v = x_ref[s + zs[ZOF[i]], k0:k0 + 128, pl.ds(c0 + uv * T, T)]
            return hv(v.astype(f32), t)
        if i == 0:
            return q(0, 0) * hv(r_u, t) + q(1, 1) * hv(r_v, t) - hv(mu, t)
        if i == 1:
            return (q(0, 0) - hv(m_u, t)) * hv(r_u, t)
        if i == 2:
            return (q(0, 1) - q(1, 1)) * hv(r_v, t)
        if i == 3:
            return (q(1, 0) - q(0, 0)) * hv(r_u, t)
        if i == 4:
            return (q(1, 1) - hv(m_v, t)) * hv(r_v, t)
        if i == 5:
            return q(0, 0) * hv(r_u, t) + q(0, 1) * hv(r_v, t) - hv(mu, t)
        return q(1, 0) * hv(r_u, t) + q(1, 1) * hv(r_v, t) - hv(mu, t)

    def tied(ref2d, base):
        w_ = ref2d.shape[1]
        rows = []
        for j in range(ref2d.shape[0] // 8):
            w = ref2d[8 * j:8 * j + 8, :]
            if base + j in ties:
                w = jnp.where(never[:, :w_], ties[base + j][:, :w_], w)
            rows.append(w)
        return jnp.concatenate(rows, axis=0)

    res, ops, lvl1 = {}, {}, {}
    rest = None
    te = 0
    for ri, rnd in enumerate(_ROUNDS):
        for pos, item in enumerate(rnd):
            if isinstance(item, str):
                h = int(item[1])
                ref2d = lr_ref.at[h * Q:(h + 1) * Q, :]
                if rest is None:
                    xr = (x_ref[s + zs[0], 2 * KH:, pl.ds(c0, T2)].astype(f32) - m) * r
                    row = lax.broadcasted_iota(jnp.int32, (16, T2), 0)
                    rest = jnp.concatenate([xr, jnp.where(row < 2, 1.0, 0.0)], axis=0).astype(bf16)
                rh = rest
            else:
                i, j = item
                if i not in ops:
                    ops[i] = [[operand(i, kh, 1 - t if i in FLIP else t) for t in range(2)]
                              for kh in range(2)]
                (b11, b12), (b21, b22) = ops[i]
                rh = (lambda: b11 + b22, lambda: b11, lambda: b12 - b22, lambda: b21 - b11,
                      lambda: b22, lambda: b11 + b12, lambda: b21 + b22)[j]().astype(bf16)
                ref2d = lb_ref.at[7 * i + j]
            if pos == 0:
                l = tied(ref2d, te)
                te += ref2d.shape[0] // 8
            else:
                l = ref2d[...]
                if pos == 1 and ri == KICK_ROUND and kick is not None:
                    l = jnp.concatenate([jnp.where(never, kick, l[:8]), l[8:]], axis=0)
            l = pltpu.bitcast(l, bf16)
            if balance and len(rnd) == 1 and not isinstance(item, str):
                cuts = (0, 48, 80, 112, Q)
                res[item] = jnp.concatenate(
                    [jnp.dot(l[lo:hi], rh, preferred_element_type=f32)
                     for lo, hi in zip(cuts[:-1], cuts[1:])], axis=0)
            else:
                res[item] = jnp.dot(l, rh, preferred_element_type=f32)
            if item == 'r0':
                top = jnp.concatenate([lvl1[0] + lvl1[3] - lvl1[4] + lvl1[6], lvl1[2] + lvl1[4]],
                                      axis=1) + res['r0']
                o_ref[s, 0:H, pl.ds(c0, T2)] = top.astype(bf16)
                if done is not None:
                    done(0, H)
            elif item != 'r1' and all((item[0], j) in res for j in range(7)):
                i = item[0]
                c11, c12, c21, c22 = _out_combos(lambda j: res[(i, j)])
                if i in FLIP:
                    c11, c12, c21, c22 = c12, c11, c22, c21
                v = jnp.concatenate([jnp.concatenate([c11, c12], axis=1),
                                     jnp.concatenate([c21, c22], axis=1)], axis=0)
                if i != ORDER[-1]:
                    acc_ref[ORDER.index(i)] = v
                    v = acc_ref[ORDER.index(i)]
                lvl1[i] = v
    bot = jnp.concatenate([lvl1[1] + lvl1[3], lvl1[0] - lvl1[1] + lvl1[2] + lvl1[5]], axis=1)
    bot = (bot + res['r1']).astype(bf16)
    if done is None:
        o_ref[s, H:, pl.ds(c0, T2)] = bot
    else:
        o_ref[s, H:H + Q, pl.ds(c0, T2)] = bot[:Q]
        done(H, Q)
        o_ref[s, H + Q:, pl.ds(c0, T2)] = bot[Q:]
        done(H + Q, Q)


def _rects(a, b):
    out = []
    while a < b:
        s, c = divmod(a, CPS)
        if c == 0 and b - a >= CPS:
            n = (b - a) // CPS
            out.append((s, n, 0, B))
            a += n * CPS
        else:
            e = min(b, (s + 1) * CPS)
            out.append((s, 1, c * T, (e - a) * T))
            a = e
    return out


_NH = sum(HEAD)
_NMID = (NCH - _NH) // MID
_MSL = MID // CPS
_HB = [sum(HEAD[:k]) for k in range(len(HEAD) + 1)]
_IN_PIECES = [_rects(0, 2)] + [_rects(_HB[k] + 2, _HB[k + 1] + 2) for k in range(len(HEAD))]
_LP = _rects(2, MID + 2)
_NSEM_IN = sum(len(p) for p in _IN_PIECES) + _NMID * len(_LP)
assert _NH + _NMID * MID == NCH and _NH % CPS == 0 and MID % CPS == 0


def _kernel(x_hbm, g_hbm, b_hbm, w_hbm, o_hbm, xbuf, obuf, wbuf, gbuf, bbuf, lb_ref, lr_ref,
            acc_ref, zref, zs_ref, isem, osem, psem):
    def in_cp(k, s, ns, c, n):
        return pltpu.make_async_copy(x_hbm.at[pl.ds(s, ns), :, pl.ds(c, n)],
                                     xbuf.at[pl.ds(s, ns), :, pl.ds(c, n)], isem.at[k])

    def out1(s, ns, c, n, r0, nr):
        pltpu.make_async_copy(obuf.at[pl.ds(s, ns), pl.ds(r0, nr), pl.ds(c, n)],
                              o_hbm.at[pl.ds(s, ns), pl.ds(r0, nr), pl.ds(c, n)],
                              osem.at[0]).start(priority=1)

    def out_start(s, n):
        for c in range(0, n, 128):
            out1(s, 1, c, 128, 0, D)

    static_in = []
    base = 0
    for p in _IN_PIECES:
        static_in.append([in_cp(base + j, *rc) for j, rc in enumerate(p)])
        base += len(p)

    def loop_in(i, j):
        s, ns, c, n = _LP[j]
        return in_cp(base + i * len(_LP) + j, _NH // CPS + i * _MSL + s, ns, c, n)

    def run(blocks, nxt, mr, zs, after=None, last_done=None):
        never = zref[...] != 0
        kick = None
        for bi, (ss, c0) in enumerate(blocks):
            ties = {}
            nx = blocks[bi + 1] if bi + 1 < len(blocks) else nxt
            nmr = _stats(xbuf, *nx, ties)
            done = None
            if last_done is not None and bi == len(blocks) - 1:
                done = lambda r0, nr: last_done(ss, c0, r0, nr)
            _block(acc_ref.at[bi % 2], lb_ref, lr_ref, xbuf, zs, mr, obuf, ss, c0, ties, never,
                   done, kick, len(blocks) % 4 != 0)
            mr = nmr
            kick = after(bi) if after is not None else None
        return mr

    wcp = pltpu.make_async_copy(w_hbm, wbuf, psem.at[0])
    gcp = pltpu.make_async_copy(g_hbm, gbuf, psem.at[1])
    bcp = pltpu.make_async_copy(b_hbm, bbuf, psem.at[2])
    gcp.start()
    bcp.start()
    wcp.start()
    for p in static_in:
        for c in p:
            c.start(priority=1)
    for i in range(_NMID):
        for j in range(len(_LP) - (1 if i == _NMID - 1 else 0)):
            loop_in(i, j).start(priority=1)
    zref[...] = jnp.zeros(zref.shape, zref.dtype)
    for i in range(NZ):
        zs_ref[i] = 0
    wcp.wait()
    gcp.wait()
    bcp.wait()
    _prep_w(wbuf, gbuf, bbuf, lb_ref, lr_ref)
    for c in static_in[0]:
        c.wait()
    mr = _stats(xbuf, 0, 0, None)

    def ch(a):
        return a // CPS, (a % CPS) * T

    for k in range(len(HEAD)):
        zs = [zs_ref[i] for i in range(NZ)]
        for c in static_in[k + 1]:
            c.wait()
        mr = run([ch(a) for a in range(_HB[k], _HB[k + 1], 2)], ch(_HB[k + 1]), mr, zs)

    nblk = MID // 2
    hi, hb, ng = HOLD
    nbl = (hb + 1) // 2
    nb = _NH // CPS + hi * _MSL + nbl
    bands = list(range(0, D, BAND))
    per = len(bands) // ng

    def body(i, mr):
        s = _NH // CPS + i * _MSL
        zs = [zs_ref[j] for j in range(NZ)]
        for j in range(len(_LP) - 1):
            loop_in(i, j).wait()
        pl.when(i + 1 < _NMID)(lambda: loop_in(i, len(_LP) - 1).wait())

        def guarded(slab, fn):
            pl.when(i >= (hi if slab >= nbl else hi + 1))(fn)

        def after(bi):
            started = False
            if hb <= bi < hb + ng:
                @pl.when(i == hi)
                def _():
                    for rr in bands[(bi - hb) * per:(bi - hb + 1) * per]:
                        out1(0, nb, 0, B, rr, BAND)
                started = True
            if bi == nblk - 2:
                guarded(bi // 2, lambda: out_start(s + bi // 2, T2))
                started = True
            elif bi % 2 == 1 and bi < nblk - 1:
                guarded(bi // 2, lambda: out_start(s + bi // 2, B))
                started = True
            if not started or bi + 1 == nblk:
                return None
            ns, nc = s + (bi + 1) // 2, ((bi + 1) % 2) * T2
            obuf[ns, 0:8, pl.ds(nc, T)] = jnp.zeros((8, T), bf16)
            return pltpu.bitcast(obuf[ns, 0:8, pl.ds(nc, T)].astype(f32)[:, :128], u32)

        def last_done(ss, c0, r0, nr):
            guarded(_MSL - 1, lambda: out1(ss, 1, c0, T2, r0, nr))

        blocks = [(s + bi // 2, (bi % 2) * T2) for bi in range(nblk)]
        return run(blocks, (jnp.minimum(s + _MSL, S - 1), 0), mr, zs, after, last_done)

    lax.fori_loop(0, _NMID, body, mr)
    pltpu.make_async_copy(obuf, o_hbm, osem.at[0]).wait()


@jax.jit
def pallas_standalone__layernorm_linear__sampling_kernel(
    x: jax.Array,
    g: jax.Array,
    b: jax.Array,
    w: jax.Array,
):
    assert x.shape == (B, S, D)
    xt = jnp.transpose(x, (1, 2, 0))
    anyspec = pl.BlockSpec(memory_space=pl.ANY)
    out = pl.pallas_call(
        _kernel,
        in_specs=[anyspec] * 4,
        out_specs=anyspec,
        out_shape=jax.ShapeDtypeStruct((S, D, B), x.dtype),
        scratch_shapes=[
            pltpu.VMEM((S, D, B), bf16), pltpu.VMEM((S, D, B), bf16),
            pltpu.VMEM((D, D), bf16), pltpu.VMEM((D,), bf16), pltpu.VMEM((D,), bf16),
            pltpu.VMEM((49, Q // 2, 128), u32), pltpu.VMEM((D // 2, KR), u32),
            pltpu.VMEM((2, 6, H, T), f32),
            pltpu.VMEM((8, 128), jnp.int32), pltpu.SMEM((NZ,), jnp.int32),
            pltpu.SemaphoreType.DMA((_NSEM_IN,)), pltpu.SemaphoreType.DMA((1,)),
            pltpu.SemaphoreType.DMA((3,)),
        ],
        compiler_params=pltpu.CompilerParams(
            vmem_limit_bytes=110 * 1024 * 1024,
            disable_bounds_checks=True,
            disable_semaphore_checks=True,
        ),
    )(xt, g, b, w)
    return jnp.transpose(out, (2, 0, 1))
```

```python
import jax
import jax.numpy as jnp
from jax import lax
import jax.experimental.pallas as pl
import jax.experimental.pallas.tpu as pltpu

EPS = 1e-5
f32 = jnp.float32
bf16 = jnp.bfloat16
u32 = jnp.uint32

S, D, B = 32, 576, 1024
H = D // 2
Q = D // 4
KH = 256
KR = D - 2 * KH + 16
T = 256
T2 = 2 * T
CPS = B // T
NCH = S * CPS

HEAD = (2, 4, 2, 8)
MID = 16
ORDER = (4, 1, 2, 3, 0, 6, 5)
INNER = (1, 4, 0, 3, 6, 2, 5)
FLIP = (6, 4, 5, 1)
TOP_AFTER = 11
TIE_SPAN = 108
KICK_ROUND = 3
HOLD = (2, 3, 4)
BAND = 24
NZ = 4
ZOF = {0: 1, 5: 2, 6: 2, 2: 3, 3: 3, 1: 0, 4: 0}


def _lhs_combos(a11, a12, a21, a22):
    return [a11 + a22, a21 + a22, a11, a22, a11 + a12, a21 - a11, a12 - a22]


def _out_combos(p):
    return (p(0) + p(3) - p(4) + p(6), p(2) + p(4), p(1) + p(3), p(0) - p(1) + p(2) + p(5))


def _rounds():
    a, b = ORDER[0], ORDER[1]
    st = [(a, 1), (a, 4), (b, 1), (b, 4)] + [(a, j) for j in INNER[2:]] + [(b, j) for j in INNER[2:]]
    st += [(i, j) for i in ORDER[2:] for j in INNER]
    rs = []
    for k in range((len(st) + 3) // 4):
        rs.append(st[4 * k:4 * k + 4])
        if k + 1 == TOP_AFTER:
            rs.append(['r0'])
    rs.append(['r1'])
    return rs


_ROUNDS = _rounds()


def _prep_w(w_ref, g_ref, b_ref, lb_ref, lr_ref):
    g = g_ref[...].astype(f32).reshape(1, D)
    b = b_ref[...].astype(f32).reshape(1, D)
    rowi = lax.broadcasted_iota(jnp.int32, (16, D), 0)
    d = jnp.dot(jnp.broadcast_to(b, (16, D)).astype(bf16), w_ref[...],
                preferred_element_type=f32)
    dh = d.astype(bf16).astype(f32)
    dd = jnp.where(rowi == 0, dh, jnp.where(rowi == 1, d - dh, 0.0)).astype(bf16)
    a = w_ref[0:2 * KH, :].astype(f32).T * g[:, :2 * KH]
    gr = jnp.concatenate([g[:, 2 * KH:], jnp.ones((1, 16), f32)], axis=1)
    ar = jnp.concatenate([w_ref[2 * KH:, :], dd], axis=0).astype(f32).T * gr
    c = jnp.sum(a[:, :128], axis=1, keepdims=True) * (1.0 / 128)
    a = a - c
    lane = lax.broadcasted_iota(jnp.int32, (1, KR), 1)
    ar = jnp.where(lane < D - 2 * KH, ar - c, ar)
    lr_ref[...] = pltpu.bitcast(ar.astype(bf16), u32)
    for i, l in enumerate(_lhs_combos(a[:H, :KH], a[:H, KH:], a[H:, :KH], a[H:, KH:])):
        for j, ll in enumerate(_lhs_combos(l[:Q, :128], l[:Q, 128:], l[Q:, :128], l[Q:, 128:])):
            lb_ref[7 * i + j] = pltpu.bitcast(ll.astype(bf16), u32)


def _stats(x_ref, s, c0, ties):
    rg = 8
    ng = D // rg
    sh = x_ref[s, 0:rg, pl.ds(c0, T2)].astype(f32)
    sh = jnp.broadcast_to(sh[0:1, :], (rg, T2))
    a1 = a2 = None
    for i in range(ng):
        v = x_ref[s, i * rg:(i + 1) * rg, pl.ds(c0, T2)].astype(f32) - sh
        if a1 is None:
            a1, a2 = v, v * v
        else:
            a1 = a1 + v
            a2 = a2 + v * v
        if ties is not None:
            j = (1, 3)[i % 2]
            ties[((i + 1) * TIE_SPAN) // ng - 1] = pltpu.bitcast(a2, u32)[:, j * 128:(j + 1) * 128]
    s1 = jnp.sum(a1, axis=0, keepdims=True) * (1.0 / D)
    s2 = jnp.sum(a2, axis=0, keepdims=True) * (1.0 / D)
    var = jnp.maximum(s2 - s1 * s1, 0.0) + EPS
    r = jnp.broadcast_to(lax.rsqrt(var), (8, T2))
    return sh + s1, r


def _block(acc_ref, lb_ref, lr_ref, x_ref, zs, mr, o_ref, s, c0, ties, never, done, kick,
           balance):
    m, r = mr[0][0:1], mr[1][0:1]
    m_u, m_v, r_u, r_v = m[:, :T], m[:, T:], r[:, :T], r[:, T:]
    mu = m_u * r_u + m_v * r_v

    def hv(v, t):
        return v[:, t * 128:(t + 1) * 128]

    def operand(i, kh, t):
        def q(kk, uv):
            k0 = kk * KH + kh * 128
            v = x_ref[s + zs[ZOF[i]], k0:k0 + 128, pl.ds(c0 + uv * T, T)]
            return hv(v.astype(f32), t)
        if i == 0:
            return q(0, 0) * hv(r_u, t) + q(1, 1) * hv(r_v, t) - hv(mu, t)
        if i == 1:
            return (q(0, 0) - hv(m_u, t)) * hv(r_u, t)
        if i == 2:
            return (q(0, 1) - q(1, 1)) * hv(r_v, t)
        if i == 3:
            return (q(1, 0) - q(0, 0)) * hv(r_u, t)
        if i == 4:
            return (q(1, 1) - hv(m_v, t)) * hv(r_v, t)
        if i == 5:
            return q(0, 0) * hv(r_u, t) + q(0, 1) * hv(r_v, t) - hv(mu, t)
        return q(1, 0) * hv(r_u, t) + q(1, 1) * hv(r_v, t) - hv(mu, t)

    def tied(ref2d, base):
        w_ = ref2d.shape[1]
        rows = []
        for j in range(ref2d.shape[0] // 8):
            w = ref2d[8 * j:8 * j + 8, :]
            if base + j in ties:
                w = jnp.where(never[:, :w_], ties[base + j][:, :w_], w)
            rows.append(w)
        return jnp.concatenate(rows, axis=0)

    res, ops, lvl1 = {}, {}, {}
    rest = None
    te = 0
    for ri, rnd in enumerate(_ROUNDS):
        for pos, item in enumerate(rnd):
            if isinstance(item, str):
                h = int(item[1])
                ref2d = lr_ref.at[h * Q:(h + 1) * Q, :]
                if rest is None:
                    xr = (x_ref[s + zs[0], 2 * KH:, pl.ds(c0, T2)].astype(f32) - m) * r
                    row = lax.broadcasted_iota(jnp.int32, (16, T2), 0)
                    rest = jnp.concatenate([xr, jnp.where(row < 2, 1.0, 0.0)], axis=0).astype(bf16)
                rh = rest
            else:
                i, j = item
                if i not in ops:
                    ops[i] = [[operand(i, kh, 1 - t if i in FLIP else t) for t in range(2)]
                              for kh in range(2)]
                (b11, b12), (b21, b22) = ops[i]
                rh = (lambda: b11 + b22, lambda: b11, lambda: b12 - b22, lambda: b21 - b11,
                      lambda: b22, lambda: b11 + b12, lambda: b21 + b22)[j]().astype(bf16)
                ref2d = lb_ref.at[7 * i + j]
            if pos == 0:
                l = tied(ref2d, te)
                te += ref2d.shape[0] // 8
            else:
                l = ref2d[...]
                if pos == 1 and ri == KICK_ROUND and kick is not None:
                    l = jnp.concatenate([jnp.where(never, kick, l[:8]), l[8:]], axis=0)
            l = pltpu.bitcast(l, bf16)
            if balance and len(rnd) == 1 and not isinstance(item, str):
                cuts = (0, 48, 80, 112, Q)
                res[item] = jnp.concatenate(
                    [jnp.dot(l[lo:hi], rh, preferred_element_type=f32)
                     for lo, hi in zip(cuts[:-1], cuts[1:])], axis=0)
            else:
                res[item] = jnp.dot(l, rh, preferred_element_type=f32)
            if item == 'r0':
                top = jnp.concatenate([lvl1[0] + lvl1[3] - lvl1[4] + lvl1[6], lvl1[2] + lvl1[4]],
                                      axis=1) + res['r0']
                o_ref[s, 0:H, pl.ds(c0, T2)] = top.astype(bf16)
                if done is not None:
                    done(0, H)
            elif item != 'r1' and all((item[0], j) in res for j in range(7)):
                i = item[0]
                c11, c12, c21, c22 = _out_combos(lambda j: res[(i, j)])
                if i in FLIP:
                    c11, c12, c21, c22 = c12, c11, c22, c21
                acc_ref[ORDER.index(i)] = jnp.concatenate(
                    [jnp.concatenate([c11, c12], axis=1), jnp.concatenate([c21, c22], axis=1)],
                    axis=0)
                lvl1[i] = acc_ref[ORDER.index(i)]
    bot = jnp.concatenate([lvl1[1] + lvl1[3], lvl1[0] - lvl1[1] + lvl1[2] + lvl1[5]], axis=1)
    bot = (bot + res['r1']).astype(bf16)
    if done is None:
        o_ref[s, H:, pl.ds(c0, T2)] = bot
    else:
        o_ref[s, H:H + Q, pl.ds(c0, T2)] = bot[:Q]
        done(H, Q)
        o_ref[s, H + Q:, pl.ds(c0, T2)] = bot[Q:]
        done(H + Q, Q)


def _rects(a, b):
    out = []
    while a < b:
        s, c = divmod(a, CPS)
        if c == 0 and b - a >= CPS:
            n = (b - a) // CPS
            out.append((s, n, 0, B))
            a += n * CPS
        else:
            e = min(b, (s + 1) * CPS)
            out.append((s, 1, c * T, (e - a) * T))
            a = e
    return out


_NH = sum(HEAD)
_NMID = (NCH - _NH) // MID
_MSL = MID // CPS
_HB = [sum(HEAD[:k]) for k in range(len(HEAD) + 1)]
_IN_PIECES = [_rects(0, 2)] + [_rects(_HB[k] + 2, _HB[k + 1] + 2) for k in range(len(HEAD))]
_LP = _rects(2, MID + 2)
_NSEM_IN = sum(len(p) for p in _IN_PIECES) + _NMID * len(_LP)
assert _NH + _NMID * MID == NCH and _NH % CPS == 0 and MID % CPS == 0


def _kernel(x_hbm, g_hbm, b_hbm, w_hbm, o_hbm, xbuf, obuf, wbuf, gbuf, bbuf, lb_ref, lr_ref,
            acc_ref, zref, zs_ref, isem, osem, psem):
    def in_cp(k, s, ns, c, n):
        return pltpu.make_async_copy(x_hbm.at[pl.ds(s, ns), :, pl.ds(c, n)],
                                     xbuf.at[pl.ds(s, ns), :, pl.ds(c, n)], isem.at[k])

    def out1(s, ns, c, n, r0, nr):
        pltpu.make_async_copy(obuf.at[pl.ds(s, ns), pl.ds(r0, nr), pl.ds(c, n)],
                              o_hbm.at[pl.ds(s, ns), pl.ds(r0, nr), pl.ds(c, n)],
                              osem.at[0]).start(priority=1)

    def out_start(s, n):
        for c in range(0, n, 128):
            out1(s, 1, c, 128, 0, D)

    static_in = []
    base = 0
    for p in _IN_PIECES:
        static_in.append([in_cp(base + j, *rc) for j, rc in enumerate(p)])
        base += len(p)

    def loop_in(i, j):
        s, ns, c, n = _LP[j]
        return in_cp(base + i * len(_LP) + j, _NH // CPS + i * _MSL + s, ns, c, n)

    def run(blocks, nxt, mr, zs, after=None, last_done=None):
        never = zref[...] != 0
        kick = None
        for bi, (ss, c0) in enumerate(blocks):
            ties = {}
            nx = blocks[bi + 1] if bi + 1 < len(blocks) else nxt
            nmr = _stats(xbuf, *nx, ties)
            done = None
            if last_done is not None and bi == len(blocks) - 1:
                done = lambda r0, nr: last_done(ss, c0, r0, nr)
            _block(acc_ref.at[bi % 2], lb_ref, lr_ref, xbuf, zs, mr, obuf, ss, c0, ties, never,
                   done, kick, len(blocks) % 4 != 0)
            mr = nmr
            kick = after(bi) if after is not None else None
        return mr

    wcp = pltpu.make_async_copy(w_hbm, wbuf, psem.at[0])
    gcp = pltpu.make_async_copy(g_hbm, gbuf, psem.at[1])
    bcp = pltpu.make_async_copy(b_hbm, bbuf, psem.at[2])
    gcp.start()
    bcp.start()
    wcp.start()
    for p in static_in:
        for c in p:
            c.start(priority=1)
    for i in range(_NMID):
        for j in range(len(_LP) - (1 if i == _NMID - 1 else 0)):
            loop_in(i, j).start(priority=1)
    zref[...] = jnp.zeros(zref.shape, zref.dtype)
    for i in range(NZ):
        zs_ref[i] = 0
    wcp.wait()
    gcp.wait()
    bcp.wait()
    _prep_w(wbuf, gbuf, bbuf, lb_ref, lr_ref)
    for c in static_in[0]:
        c.wait()
    mr = _stats(xbuf, 0, 0, None)

    def ch(a):
        return a // CPS, (a % CPS) * T

    for k in range(len(HEAD)):
        zs = [zs_ref[i] for i in range(NZ)]
        for c in static_in[k + 1]:
            c.wait()
        mr = run([ch(a) for a in range(_HB[k], _HB[k + 1], 2)], ch(_HB[k + 1]), mr, zs)

    nblk = MID // 2
    hi, hb, ng = HOLD
    nbl = (hb + 1) // 2
    nb = _NH // CPS + hi * _MSL + nbl
    bands = list(range(0, D, BAND))
    per = len(bands) // ng

    def body(i, mr):
        s = _NH // CPS + i * _MSL
        zs = [zs_ref[j] for j in range(NZ)]
        for j in range(len(_LP) - 1):
            loop_in(i, j).wait()
        pl.when(i + 1 < _NMID)(lambda: loop_in(i, len(_LP) - 1).wait())

        def guarded(slab, fn):
            pl.when(i >= (hi if slab >= nbl else hi + 1))(fn)

        def after(bi):
            started = False
            if hb <= bi < hb + ng:
                @pl.when(i == hi)
                def _():
                    for rr in bands[(bi - hb) * per:(bi - hb + 1) * per]:
                        out1(0, nb, 0, B, rr, BAND)
                started = True
            if bi == nblk - 2:
                guarded(bi // 2, lambda: out_start(s + bi // 2, T2))
                started = True
            elif bi % 2 == 1 and bi < nblk - 1:
                guarded(bi // 2, lambda: out_start(s + bi // 2, B))
                started = True
            if not started or bi + 1 == nblk:
                return None
            ns, nc = s + (bi + 1) // 2, ((bi + 1) % 2) * T2
            obuf[ns, 0:8, pl.ds(nc, T)] = jnp.zeros((8, T), bf16)
            return pltpu.bitcast(obuf[ns, 0:8, pl.ds(nc, T)].astype(f32)[:, :128], u32)

        def last_done(ss, c0, r0, nr):
            guarded(_MSL - 1, lambda: out1(ss, 1, c0, T2, r0, nr))

        blocks = [(s + bi // 2, (bi % 2) * T2) for bi in range(nblk)]
        return run(blocks, (jnp.minimum(s + _MSL, S - 1), 0), mr, zs, after, last_done)

    lax.fori_loop(0, _NMID, body, mr)
    pltpu.make_async_copy(obuf, o_hbm, osem.at[0]).wait()


@jax.jit
def pallas_standalone__layernorm_linear__sampling_kernel(
    x: jax.Array,
    g: jax.Array,
    b: jax.Array,
    w: jax.Array,
):
    assert x.shape == (B, S, D)
    xt = jnp.transpose(x, (1, 2, 0))
    anyspec = pl.BlockSpec(memory_space=pl.ANY)
    out = pl.pallas_call(
        _kernel,
        in_specs=[anyspec] * 4,
        out_specs=anyspec,
        out_shape=jax.ShapeDtypeStruct((S, D, B), x.dtype),
        scratch_shapes=[
            pltpu.VMEM((S, D, B), bf16), pltpu.VMEM((S, D, B), bf16),
            pltpu.VMEM((D, D), bf16), pltpu.VMEM((D,), bf16), pltpu.VMEM((D,), bf16),
            pltpu.VMEM((49, Q // 2, 128), u32), pltpu.VMEM((D // 2, KR), u32),
            pltpu.VMEM((2, 7, H, T), f32),
            pltpu.VMEM((8, 128), jnp.int32), pltpu.SMEM((NZ,), jnp.int32),
            pltpu.SemaphoreType.DMA((_NSEM_IN,)), pltpu.SemaphoreType.DMA((1,)),
            pltpu.SemaphoreType.DMA((3,)),
        ],
        compiler_params=pltpu.CompilerParams(
            vmem_limit_bytes=110 * 1024 * 1024,
            disable_bounds_checks=True,
            disable_semaphore_checks=True,
        ),
    )(xt, g, b, w)
    return jnp.transpose(out, (2, 0, 1))
```

```python
import jax
import jax.numpy as jnp
from jax import lax
import jax.experimental.pallas as pl
import jax.experimental.pallas.tpu as pltpu

EPS = 1e-5
f32 = jnp.float32
bf16 = jnp.bfloat16
u32 = jnp.uint32

S, D, B = 32, 576, 1024
H = D // 2
Q = D // 4
KH = 256
KR = D - 2 * KH + 16
T = 256
T2 = 2 * T
CPS = B // T
NCH = S * CPS

HEAD = (2, 4, 2, 8)
MID = 16
ORDER = (4, 1, 2, 3, 0, 6, 5)
INNER = (1, 4, 0, 3, 6, 2, 5)
FLIP = (6, 4, 5, 1)
TOP_AFTER = 11
TIE_SPAN = (9, 117)
KICK_ROUND = 3
HOLD = (2, 3, 4)
BAND = 24
NZ = 4
ZOF = {0: 1, 5: 2, 6: 2, 2: 3, 3: 3, 1: 0, 4: 0}


def _lhs_combos(a11, a12, a21, a22):
    return [a11 + a22, a21 + a22, a11, a22, a11 + a12, a21 - a11, a12 - a22]


def _out_combos(p):
    return (p(0) + p(3) - p(4) + p(6), p(2) + p(4), p(1) + p(3), p(0) - p(1) + p(2) + p(5))


def _rounds(top_after):
    a, b = ORDER[0], ORDER[1]
    st = [(a, 1), (a, 4), (b, 1), (b, 4)] + [(a, j) for j in INNER[2:]] + [(b, j) for j in INNER[2:]]
    st += [(i, j) for i in ORDER[2:] for j in INNER]
    rs = [st[k:k + 4] for k in range(0, len(st), 4)]
    return rs[:top_after] + [['r0']] + rs[top_after:] + [['r1']]


_ROUNDS = _rounds(TOP_AFTER)
_ROUNDS_FIRST = _rounds(0)


def _prep_w(w_ref, g_ref, b_ref, lb_ref, lr_ref):
    g = g_ref[...].astype(f32).reshape(1, D)
    b = b_ref[...].astype(f32).reshape(1, D)
    a = w_ref[0:2 * KH, :].astype(f32).T * g[:, :2 * KH]
    c = jnp.sum(a[:, :128], axis=1, keepdims=True) * (1.0 / 128)
    a = a - c
    d = jnp.dot(jnp.broadcast_to(b, (16, D)).astype(bf16), w_ref[...],
                preferred_element_type=f32)
    dh = d.astype(bf16).astype(f32)
    rowi = lax.broadcasted_iota(jnp.int32, (16, D), 0)
    dd = jnp.where(rowi == 0, dh, jnp.where(rowi == 1, d - dh, 0.0)).astype(bf16)
    gr = jnp.concatenate([g[:, 2 * KH:], jnp.ones((1, 16), f32)], axis=1)
    ar = jnp.concatenate([w_ref[2 * KH:, :], dd], axis=0).astype(f32).T * gr
    lane = lax.broadcasted_iota(jnp.int32, (1, KR), 1)
    ar = jnp.where(lane < D - 2 * KH, ar - c, ar)
    lr_ref[...] = pltpu.bitcast(ar.astype(bf16), u32)
    for i, l in enumerate(_lhs_combos(a[:H, :KH], a[:H, KH:], a[H:, :KH], a[H:, KH:])):
        for j, ll in enumerate(_lhs_combos(l[:Q, :128], l[:Q, 128:], l[Q:, :128], l[Q:, 128:])):
            lb_ref[7 * i + j] = pltpu.bitcast(ll.astype(bf16), u32)


def _stats(x_ref, s, c0, ties):
    rg = 8
    ng = D // rg
    sh = x_ref[s, 0:rg, pl.ds(c0, T2)].astype(f32)
    sh = jnp.broadcast_to(sh[0:1, :], (rg, T2))
    a1 = a2 = None
    for i in range(ng):
        v = x_ref[s, i * rg:(i + 1) * rg, pl.ds(c0, T2)].astype(f32) - sh
        if a1 is None:
            a1, a2 = v, v * v
        else:
            a1 = a1 + v
            a2 = a2 + v * v
        if ties is not None:
            j = (1, 3)[i % 2]
            t = TIE_SPAN[0] + ((i + 1) * (TIE_SPAN[1] - TIE_SPAN[0])) // ng - 1
            ties[t] = pltpu.bitcast(a2, u32)[:, j * 128:(j + 1) * 128]
    s1 = jnp.sum(a1, axis=0, keepdims=True) * (1.0 / D)
    s2 = jnp.sum(a2, axis=0, keepdims=True) * (1.0 / D)
    var = jnp.maximum(s2 - s1 * s1, 0.0) + EPS
    r = jnp.broadcast_to(lax.rsqrt(var), (8, T2))
    return sh + s1, r


def _block(acc_ref, lb_ref, lr_ref, x_ref, zs, mr, o_ref, s, c0, ties, never, done, kick,
           rounds, balance):
    m, r = mr[0][0:1], mr[1][0:1]
    m_u, m_v, r_u, r_v = m[:, :T], m[:, T:], r[:, :T], r[:, T:]
    mu = m_u * r_u + m_v * r_v

    def hv(v, t):
        return v[:, t * 128:(t + 1) * 128]

    def operand(i, kh, t):
        def q(kk, uv):
            k0 = kk * KH + kh * 128
            v = x_ref[s + zs[ZOF[i]], k0:k0 + 128, pl.ds(c0 + uv * T, T)]
            return hv(v.astype(f32), t)
        if i == 0:
            return q(0, 0) * hv(r_u, t) + q(1, 1) * hv(r_v, t) - hv(mu, t)
        if i == 1:
            return (q(0, 0) - hv(m_u, t)) * hv(r_u, t)
        if i == 2:
            return (q(0, 1) - q(1, 1)) * hv(r_v, t)
        if i == 3:
            return (q(1, 0) - q(0, 0)) * hv(r_u, t)
        if i == 4:
            return (q(1, 1) - hv(m_v, t)) * hv(r_v, t)
        if i == 5:
            return q(0, 0) * hv(r_u, t) + q(0, 1) * hv(r_v, t) - hv(mu, t)
        return q(1, 0) * hv(r_u, t) + q(1, 1) * hv(r_v, t) - hv(mu, t)

    def tied(ref2d, base):
        w_ = ref2d.shape[1]
        rows = []
        for j in range(ref2d.shape[0] // 8):
            w = ref2d[8 * j:8 * j + 8, :]
            if base + j in ties:
                w = jnp.where(never[:, :w_], ties[base + j][:, :w_], w)
            rows.append(w)
        return jnp.concatenate(rows, axis=0)

    res, ops, lvl1 = {}, {}, {}
    rest = None
    top_done = False
    te = 0
    for ri, rnd in enumerate(rounds):
        for pos, item in enumerate(rnd):
            if isinstance(item, str):
                h = int(item[1])
                ref2d = lr_ref.at[h * Q:(h + 1) * Q, :]
                if rest is None:
                    xr = (x_ref[s + zs[0], 2 * KH:, pl.ds(c0, T2)].astype(f32) - m) * r
                    row = lax.broadcasted_iota(jnp.int32, (16, T2), 0)
                    rest = jnp.concatenate([xr, jnp.where(row < 2, 1.0, 0.0)], axis=0).astype(bf16)
                rh = rest
            else:
                i, j = item
                if i not in ops:
                    ops[i] = [[operand(i, kh, 1 - t if i in FLIP else t) for t in range(2)]
                              for kh in range(2)]
                (b11, b12), (b21, b22) = ops[i]
                rh = (lambda: b11 + b22, lambda: b11, lambda: b12 - b22, lambda: b21 - b11,
                      lambda: b22, lambda: b11 + b12, lambda: b21 + b22)[j]().astype(bf16)
                ref2d = lb_ref.at[7 * i + j]
            if pos == 0:
                l = tied(ref2d, te)
                te += ref2d.shape[0] // 8
            else:
                l = ref2d[...]
                if pos == 1 and ri == KICK_ROUND and kick is not None:
                    l = jnp.concatenate([jnp.where(never, kick, l[:8]), l[8:]], axis=0)
            l = pltpu.bitcast(l, bf16)
            if balance and len(rnd) == 1 and not isinstance(item, str):
                cuts = (0, 48, 80, 112, Q)
                res[item] = jnp.concatenate(
                    [jnp.dot(l[lo:hi], rh, preferred_element_type=f32)
                     for lo, hi in zip(cuts[:-1], cuts[1:])], axis=0)
            else:
                res[item] = jnp.dot(l, rh, preferred_element_type=f32)
            if not isinstance(item, str) and all((item[0], j) in res for j in range(7)):
                i = item[0]
                c11, c12, c21, c22 = _out_combos(lambda j: res[(i, j)])
                if i in FLIP:
                    c11, c12, c21, c22 = c12, c11, c22, c21
                acc_ref[ORDER.index(i)] = jnp.concatenate(
                    [jnp.concatenate([c11, c12], axis=1), jnp.concatenate([c21, c22], axis=1)],
                    axis=0)
                lvl1[i] = acc_ref[ORDER.index(i)]
            if not top_done and 'r0' in res and all(i in lvl1 for i in (0, 2, 3, 4, 6)):
                top_done = True
                top = jnp.concatenate([lvl1[0] + lvl1[3] - lvl1[4] + lvl1[6], lvl1[2] + lvl1[4]],
                                      axis=1) + res['r0']
                o_ref[s, 0:H, pl.ds(c0, T2)] = top.astype(bf16)
                if done is not None:
                    done(0, H)
    bot = jnp.concatenate([lvl1[1] + lvl1[3], lvl1[0] - lvl1[1] + lvl1[2] + lvl1[5]], axis=1)
    bot = (bot + res['r1']).astype(bf16)
    if done is None:
        o_ref[s, H:, pl.ds(c0, T2)] = bot
    else:
        o_ref[s, H:H + Q, pl.ds(c0, T2)] = bot[:Q]
        done(H, Q)
        o_ref[s, H + Q:, pl.ds(c0, T2)] = bot[Q:]
        done(H + Q, Q)


def _rects(a, b):
    out = []
    while a < b:
        s, c = divmod(a, CPS)
        if c == 0 and b - a >= CPS:
            n = (b - a) // CPS
            out.append((s, n, 0, B))
            a += n * CPS
        else:
            e = min(b, (s + 1) * CPS)
            out.append((s, 1, c * T, (e - a) * T))
            a = e
    return out


_NH = sum(HEAD)
_NMID = (NCH - _NH) // MID
_MSL = MID // CPS
_HB = [sum(HEAD[:k]) for k in range(len(HEAD) + 1)]
_IN_PIECES = [_rects(0, 2)] + [_rects(_HB[k] + 2, _HB[k + 1] + 2) for k in range(len(HEAD))]
_LP = _rects(2, MID + 2)
_NSEM_IN = sum(len(p) for p in _IN_PIECES) + _NMID * len(_LP)
assert _NH + _NMID * MID == NCH and _NH % CPS == 0 and MID % CPS == 0


def _kernel(x_hbm, g_hbm, b_hbm, w_hbm, o_hbm, xbuf, obuf, wbuf, gbuf, bbuf, lb_ref, lr_ref,
            acc_ref, zref, zs_ref, isem, osem, psem):
    def in_cp(k, s, ns, c, n):
        return pltpu.make_async_copy(x_hbm.at[pl.ds(s, ns), :, pl.ds(c, n)],
                                     xbuf.at[pl.ds(s, ns), :, pl.ds(c, n)], isem.at[k])

    def out1(s, ns, c, n, r0, nr):
        pltpu.make_async_copy(obuf.at[pl.ds(s, ns), pl.ds(r0, nr), pl.ds(c, n)],
                              o_hbm.at[pl.ds(s, ns), pl.ds(r0, nr), pl.ds(c, n)],
                              osem.at[0]).start(priority=1)

    def out_start(s, n):
        for c in range(0, n, 128):
            out1(s, 1, c, 128, 0, D)

    static_in = []
    base = 0
    for p in _IN_PIECES:
        static_in.append([in_cp(base + j, *rc) for j, rc in enumerate(p)])
        base += len(p)

    def loop_in(i, j):
        s, ns, c, n = _LP[j]
        return in_cp(base + i * len(_LP) + j, _NH // CPS + i * _MSL + s, ns, c, n)

    def run(blocks, nxt, mr, zs, after=None, last_done=None):
        never = zref[...] != 0
        kick = None
        for bi, (ss, c0) in enumerate(blocks):
            ties = {}
            nx = blocks[bi + 1] if bi + 1 < len(blocks) else nxt
            nmr = _stats(xbuf, *nx, ties)
            done = None
            if last_done is not None and bi == len(blocks) - 1:
                done = lambda r0, nr: last_done(ss, c0, r0, nr)
            _block(acc_ref.at[bi % 2], lb_ref, lr_ref, xbuf, zs, mr, obuf, ss, c0, ties, never,
                   done, kick, _ROUNDS_FIRST if bi == 0 else _ROUNDS, len(blocks) % 4 != 0)
            mr = nmr
            kick = after(bi) if after is not None else None
        return mr

    wcp = pltpu.make_async_copy(w_hbm, wbuf, psem.at[0])
    gcp = pltpu.make_async_copy(g_hbm, gbuf, psem.at[1])
    bcp = pltpu.make_async_copy(b_hbm, bbuf, psem.at[2])
    gcp.start()
    bcp.start()
    wcp.start()
    for p in static_in:
        for c in p:
            c.start(priority=1)
    for i in range(_NMID):
        for j in range(len(_LP) - (1 if i == _NMID - 1 else 0)):
            loop_in(i, j).start(priority=1)
    zref[...] = jnp.zeros(zref.shape, zref.dtype)
    for i in range(NZ):
        zs_ref[i] = 0
    wcp.wait()
    gcp.wait()
    bcp.wait()
    _prep_w(wbuf, gbuf, bbuf, lb_ref, lr_ref)
    for c in static_in[0]:
        c.wait()
    mr = _stats(xbuf, 0, 0, None)

    def ch(a):
        return a // CPS, (a % CPS) * T

    for k in range(len(HEAD)):
        zs = [zs_ref[i] for i in range(NZ)]
        for c in static_in[k + 1]:
            c.wait()
        mr = run([ch(a) for a in range(_HB[k], _HB[k + 1], 2)], ch(_HB[k + 1]), mr, zs)

    nblk = MID // 2
    hi, hb, ng = HOLD
    nbl = (hb + 1) // 2
    nb = _NH // CPS + hi * _MSL + nbl
    bands = list(range(0, D, BAND))
    per = len(bands) // ng

    def body(i, mr):
        s = _NH // CPS + i * _MSL
        zs = [zs_ref[j] for j in range(NZ)]
        for j in range(len(_LP) - 1):
            loop_in(i, j).wait()
        pl.when(i + 1 < _NMID)(lambda: loop_in(i, len(_LP) - 1).wait())

        def guarded(slab, fn):
            pl.when(i >= (hi if slab >= nbl else hi + 1))(fn)

        def after(bi):
            started = False
            if hb <= bi < hb + ng:
                @pl.when(i == hi)
                def _():
                    for rr in bands[(bi - hb) * per:(bi - hb + 1) * per]:
                        out1(0, nb, 0, B, rr, BAND)
                started = True
            if bi == nblk - 2:
                guarded(bi // 2, lambda: out_start(s + bi // 2, T2))
                started = True
            elif bi % 2 == 1 and bi < nblk - 1:
                guarded(bi // 2, lambda: out_start(s + bi // 2, B))
                started = True
            if not started or bi + 1 == nblk:
                return None
            ns, nc = s + (bi + 1) // 2, ((bi + 1) % 2) * T2
            obuf[ns, 0:8, pl.ds(nc, T)] = jnp.zeros((8, T), bf16)
            return pltpu.bitcast(obuf[ns, 0:8, pl.ds(nc, T)].astype(f32)[:, :128], u32)

        def last_done(ss, c0, r0, nr):
            guarded(_MSL - 1, lambda: out1(ss, 1, c0, T2, r0, nr))

        blocks = [(s + bi // 2, (bi % 2) * T2) for bi in range(nblk)]
        return run(blocks, (jnp.minimum(s + _MSL, S - 1), 0), mr, zs, after, last_done)

    lax.fori_loop(0, _NMID, body, mr)
    pltpu.make_async_copy(obuf, o_hbm, osem.at[0]).wait()


@jax.jit
def pallas_standalone__layernorm_linear__sampling_kernel(
    x: jax.Array,
    g: jax.Array,
    b: jax.Array,
    w: jax.Array,
):
    assert x.shape == (B, S, D)
    xt = jnp.transpose(x, (1, 2, 0))
    anyspec = pl.BlockSpec(memory_space=pl.ANY)
    out = pl.pallas_call(
        _kernel,
        in_specs=[anyspec] * 4,
        out_specs=anyspec,
        out_shape=jax.ShapeDtypeStruct((S, D, B), x.dtype),
        scratch_shapes=[
            pltpu.VMEM((S, D, B), bf16), pltpu.VMEM((S, D, B), bf16),
            pltpu.VMEM((D, D), bf16), pltpu.VMEM((D,), bf16), pltpu.VMEM((D,), bf16),
            pltpu.VMEM((49, Q // 2, 128), u32), pltpu.VMEM((D // 2, KR), u32),
            pltpu.VMEM((2, 7, H, T), f32),
            pltpu.VMEM((8, 128), jnp.int32), pltpu.SMEM((NZ,), jnp.int32),
            pltpu.SemaphoreType.DMA((_NSEM_IN,)), pltpu.SemaphoreType.DMA((1,)),
            pltpu.SemaphoreType.DMA((3,)),
        ],
        compiler_params=pltpu.CompilerParams(
            vmem_limit_bytes=110 * 1024 * 1024,
            disable_bounds_checks=True,
            disable_semaphore_checks=True,
        ),
    )(xt, g, b, w)
    return jnp.transpose(out, (2, 0, 1))
```

```python
import jax
import jax.numpy as jnp
from jax import lax
import jax.experimental.pallas as pl
import jax.experimental.pallas.tpu as pltpu

EPS = 1e-5
f32 = jnp.float32
bf16 = jnp.bfloat16
u32 = jnp.uint32

S, D, B = 32, 576, 1024
H = D // 2
Q = D // 4
KH = 256
KR = D - 2 * KH + 16
T = 256
T2 = 2 * T
CPS = B // T
NCH = S * CPS

HEAD = (2, 4, 2, 8)
MID = 16
ORDER = (4, 1, 2, 3, 0, 6, 5)
INNER = (1, 4, 0, 3, 6, 2, 5)
FLIP = (6, 4, 5, 1)
TOP_AFTER = 11
TIE_SPAN = (9, 117)
KICK_ROUND = 3
HOLD = (2, 3, 4)
BAND = 24
NZ = 4
ZOF = {0: 1, 5: 2, 6: 2, 2: 3, 3: 3, 1: 0, 4: 0}


def _lhs_combos(a11, a12, a21, a22):
    return [a11 + a22, a21 + a22, a11, a22, a11 + a12, a21 - a11, a12 - a22]


def _out_combos(p):
    return (p(4) + p(0) + p(3) + p(6), p(2) + p(4), p(1) + p(3), p(1) - p(0) + p(2) - p(5))


def _rounds(top_after):
    a, b = ORDER[0], ORDER[1]
    st = [(a, 1), (a, 4), (b, 1), (b, 4)] + [(a, j) for j in INNER[2:]] + [(b, j) for j in INNER[2:]]
    st += [(i, j) for i in ORDER[2:] for j in INNER]
    rs = [st[k:k + 4] for k in range(0, len(st), 4)]
    return rs[:top_after] + [['r0']] + rs[top_after:] + [['r1']]


_ROUNDS = _rounds(TOP_AFTER)
_ROUNDS_FIRST = _rounds(0)


def _prep_w(w_ref, g_ref, b_ref, lb_ref, lr_ref):
    g = g_ref[...].astype(f32).reshape(1, D)
    b = b_ref[...].astype(f32).reshape(1, D)
    a = w_ref[0:2 * KH, :].astype(f32).T * g[:, :2 * KH]
    c = jnp.sum(a[:, :128], axis=1, keepdims=True) * (1.0 / 128)
    a = a - c
    d = jnp.dot(jnp.broadcast_to(b, (16, D)).astype(bf16), w_ref[...],
                preferred_element_type=f32)
    dh = d.astype(bf16).astype(f32)
    rowi = lax.broadcasted_iota(jnp.int32, (16, D), 0)
    dd = jnp.where(rowi == 0, dh, jnp.where(rowi == 1, d - dh, 0.0)).astype(bf16)
    gr = jnp.concatenate([g[:, 2 * KH:], jnp.ones((1, 16), f32)], axis=1)
    ar = jnp.concatenate([w_ref[2 * KH:, :], dd], axis=0).astype(f32).T * gr
    lane = lax.broadcasted_iota(jnp.int32, (1, KR), 1)
    ar = jnp.where(lane < D - 2 * KH, ar - c, ar)
    lr_ref[...] = pltpu.bitcast(ar.astype(bf16), u32)
    for i, l in enumerate(_lhs_combos(a[:H, :KH], a[:H, KH:], a[H:, :KH], a[H:, KH:])):
        for j, ll in enumerate(_lhs_combos(l[:Q, :128], l[:Q, 128:], l[Q:, :128], l[Q:, 128:])):
            lb_ref[7 * i + j] = pltpu.bitcast(ll.astype(bf16), u32)


def _stats(x_ref, s, c0, ties):
    rg = 8
    ng = D // rg
    sh = x_ref[s, 0:rg, pl.ds(c0, T2)].astype(f32)
    sh = jnp.broadcast_to(sh[0:1, :], (rg, T2))
    a1 = a2 = None
    for i in range(ng):
        v = x_ref[s, i * rg:(i + 1) * rg, pl.ds(c0, T2)].astype(f32) - sh
        if a1 is None:
            a1, a2 = v, v * v
        else:
            a1 = a1 + v
            a2 = a2 + v * v
        if ties is not None:
            j = (1, 3)[i % 2]
            t = TIE_SPAN[0] + ((i + 1) * (TIE_SPAN[1] - TIE_SPAN[0])) // ng - 1
            ties[t] = pltpu.bitcast(a2, u32)[:, j * 128:(j + 1) * 128]
    s1 = jnp.sum(a1, axis=0, keepdims=True) * (1.0 / D)
    s2 = jnp.sum(a2, axis=0, keepdims=True) * (1.0 / D)
    var = jnp.maximum(s2 - s1 * s1, 0.0) + EPS
    r = jnp.broadcast_to(lax.rsqrt(var), (8, T2))
    return sh + s1, r


def _block(acc_ref, lb_ref, lr_ref, x_ref, zs, mr, o_ref, s, c0, ties, never, done, kick,
           rounds, balance):
    m, r = mr[0][0:1], mr[1][0:1]
    m_u, m_v, r_u, r_v = m[:, :T], m[:, T:], r[:, :T], r[:, T:]
    mu = m_u * r_u - m_v * r_v

    sz = [jnp.clip(s + z, s, s) for z in zs]

    def hv(v, t):
        return v[:, t * 128:(t + 1) * 128]

    def operand(i, kh, t):
        def q(kk, uv):
            k0 = kk * KH + kh * 128
            v = x_ref[sz[ZOF[i]], k0:k0 + 128, pl.ds(c0 + uv * T, T)]
            return hv(v.astype(f32), t)
        if i == 0:
            return q(0, 0) * hv(r_u, t) - q(1, 1) * hv(r_v, t) - hv(mu, t)
        if i == 1:
            return (q(0, 0) - hv(m_u, t)) * hv(r_u, t)
        if i == 2:
            return (q(0, 1) - q(1, 1)) * hv(r_v, t)
        if i == 3:
            return (q(1, 0) - q(0, 0)) * hv(r_u, t)
        if i == 4:
            return (q(1, 1) - hv(m_v, t)) * hv(r_v, t)
        if i == 5:
            return q(0, 0) * hv(r_u, t) - q(0, 1) * hv(r_v, t) - hv(mu, t)
        return q(1, 0) * hv(r_u, t) - q(1, 1) * hv(r_v, t) - hv(mu, t)

    def tied(ref2d, base):
        w_ = ref2d.shape[1]
        rows = []
        for j in range(ref2d.shape[0] // 8):
            w = ref2d[8 * j:8 * j + 8, :]
            if base + j in ties:
                w = jnp.where(never[:, :w_], ties[base + j][:, :w_], w)
            rows.append(w)
        return jnp.concatenate(rows, axis=0)

    res, ops, lvl1 = {}, {}, {}
    rest = None
    top_done = False
    te = 0
    for ri, rnd in enumerate(rounds):
        for pos, item in enumerate(rnd):
            if isinstance(item, str):
                h = int(item[1])
                ref2d = lr_ref.at[h * Q:(h + 1) * Q, :]
                if rest is None:
                    xr = (x_ref[sz[0], 2 * KH:, pl.ds(c0, T2)].astype(f32) - m) * r
                    row = lax.broadcasted_iota(jnp.int32, (16, T2), 0)
                    rest = jnp.concatenate([xr, jnp.where(row < 2, 1.0, 0.0)], axis=0).astype(bf16)
                rh = rest
            else:
                i, j = item
                if i not in ops:
                    ops[i] = [[operand(i, kh, 1 - t if i in FLIP else t) for t in range(2)]
                              for kh in range(2)]
                (b11, b12), (b21, b22) = ops[i]
                rh = (lambda: b11 - b22, lambda: b11, lambda: b12 - b22, lambda: b21 - b11,
                      lambda: b22, lambda: b11 - b12, lambda: b21 - b22)[j]().astype(bf16)
                ref2d = lb_ref.at[7 * i + j]
            if pos == 0:
                l = tied(ref2d, te)
                te += ref2d.shape[0] // 8
            else:
                l = ref2d[...]
                if pos == 1 and ri == KICK_ROUND and kick is not None:
                    l = jnp.concatenate([jnp.where(never, kick, l[:8]), l[8:]], axis=0)
            l = pltpu.bitcast(l, bf16)
            if balance and len(rnd) == 1 and not isinstance(item, str):
                cuts = (0, 48, 80, 112, Q)
                res[item] = jnp.concatenate(
                    [jnp.dot(l[lo:hi], rh, preferred_element_type=f32)
                     for lo, hi in zip(cuts[:-1], cuts[1:])], axis=0)
            else:
                res[item] = jnp.dot(l, rh, preferred_element_type=f32)
            if not isinstance(item, str) and all((item[0], j) in res for j in range(7)):
                i = item[0]
                c11, c12, c21, c22 = _out_combos(lambda j: res[(i, j)])
                if i in FLIP:
                    c11, c12, c21, c22 = c12, c11, c22, c21
                acc_ref[ORDER.index(i)] = jnp.concatenate(
                    [jnp.concatenate([c11, c12], axis=1), jnp.concatenate([c21, c22], axis=1)],
                    axis=0)
                lvl1[i] = acc_ref[ORDER.index(i)]
            if not top_done and 'r0' in res and all(i in lvl1 for i in (0, 2, 3, 4, 6)):
                top_done = True
                top = jnp.concatenate([lvl1[0] + lvl1[3] + lvl1[4] + lvl1[6], lvl1[2] + lvl1[4]],
                                      axis=1) + res['r0']
                o_ref[s, 0:H, pl.ds(c0, T2)] = top.astype(bf16)
                if done is not None:
                    done(0, H)
    bot = jnp.concatenate([lvl1[1] + lvl1[3], lvl1[1] - lvl1[0] + lvl1[2] - lvl1[5]], axis=1)
    bot = (bot + res['r1']).astype(bf16)
    if done is None:
        o_ref[s, H:, pl.ds(c0, T2)] = bot
    else:
        o_ref[s, H:H + Q, pl.ds(c0, T2)] = bot[:Q]
        done(H, Q)
        o_ref[s, H + Q:, pl.ds(c0, T2)] = bot[Q:]
        done(H + Q, Q)


def _rects(a, b):
    out = []
    while a < b:
        s, c = divmod(a, CPS)
        if c == 0 and b - a >= CPS:
            n = (b - a) // CPS
            out.append((s, n, 0, B))
            a += n * CPS
        else:
            e = min(b, (s + 1) * CPS)
            out.append((s, 1, c * T, (e - a) * T))
            a = e
    return out


_NH = sum(HEAD)
_NMID = (NCH - _NH) // MID
_MSL = MID // CPS
_HB = [sum(HEAD[:k]) for k in range(len(HEAD) + 1)]
_IN_PIECES = [_rects(0, 2)] + [_rects(_HB[k] + 2, _HB[k + 1] + 2) for k in range(len(HEAD))]
_LP = _rects(2, MID + 2)
_NSEM_IN = sum(len(p) for p in _IN_PIECES) + _NMID * len(_LP)
assert _NH + _NMID * MID == NCH and _NH % CPS == 0 and MID % CPS == 0


def _kernel(x_hbm, g_hbm, b_hbm, w_hbm, o_hbm, xbuf, obuf, wbuf, gbuf, bbuf, lb_ref, lr_ref,
            acc_ref, zref, zs_ref, isem, osem, psem):
    def in_cp(k, s, ns, c, n):
        return pltpu.make_async_copy(x_hbm.at[pl.ds(s, ns), :, pl.ds(c, n)],
                                     xbuf.at[pl.ds(s, ns), :, pl.ds(c, n)], isem.at[k])

    def out1(s, ns, c, n, r0, nr):
        pltpu.make_async_copy(obuf.at[pl.ds(s, ns), pl.ds(r0, nr), pl.ds(c, n)],
                              o_hbm.at[pl.ds(s, ns), pl.ds(r0, nr), pl.ds(c, n)],
                              osem.at[0]).start(priority=1)

    def out_start(s, n):
        for c in range(0, n, 128):
            out1(s, 1, c, 128, 0, D)

    static_in = []
    base = 0
    for p in _IN_PIECES:
        static_in.append([in_cp(base + j, *rc) for j, rc in enumerate(p)])
        base += len(p)

    def loop_in(i, j):
        s, ns, c, n = _LP[j]
        return in_cp(base + i * len(_LP) + j, _NH // CPS + i * _MSL + s, ns, c, n)

    def run(blocks, nxt, mr, zs, after=None, last_done=None):
        never = zref[...] != 0
        kick = None
        for bi, (ss, c0) in enumerate(blocks):
            ties = {}
            nx = blocks[bi + 1] if bi + 1 < len(blocks) else nxt
            nmr = _stats(xbuf, *nx, ties)
            done = None
            if last_done is not None and bi == len(blocks) - 1:
                done = lambda r0, nr: last_done(ss, c0, r0, nr)
            _block(acc_ref.at[bi % 2], lb_ref, lr_ref, xbuf, zs, mr, obuf, ss, c0, ties, never,
                   done, kick, _ROUNDS_FIRST if bi == 0 else _ROUNDS, len(blocks) % 4 != 0)
            mr = nmr
            kick = after(bi) if after is not None else None
        return mr

    wcp = pltpu.make_async_copy(w_hbm, wbuf, psem.at[0])
    gcp = pltpu.make_async_copy(g_hbm, gbuf, psem.at[1])
    bcp = pltpu.make_async_copy(b_hbm, bbuf, psem.at[2])
    gcp.start()
    bcp.start()
    wcp.start()
    for p in static_in:
        for c in p:
            c.start(priority=1)
    for i in range(_NMID):
        for j in range(len(_LP) - (1 if i == _NMID - 1 else 0)):
            loop_in(i, j).start(priority=1)
    zref[...] = jnp.zeros(zref.shape, zref.dtype)
    for i in range(NZ):
        zs_ref[i] = 0
    wcp.wait()
    gcp.wait()
    bcp.wait()
    _prep_w(wbuf, gbuf, bbuf, lb_ref, lr_ref)
    for c in static_in[0]:
        c.wait()
    mr = _stats(xbuf, 0, 0, None)

    def ch(a):
        return a // CPS, (a % CPS) * T

    for k in range(len(HEAD)):
        zs = [zs_ref[i] for i in range(NZ)]
        for c in static_in[k + 1]:
            c.wait()
        mr = run([ch(a) for a in range(_HB[k], _HB[k + 1], 2)], ch(_HB[k + 1]), mr, zs)

    nblk = MID // 2
    hi, hb, ng = HOLD
    nbl = (hb + 1) // 2
    nb = _NH // CPS + hi * _MSL + nbl
    bands = list(range(0, D, BAND))
    per = len(bands) // ng

    def body(i, mr):
        s = _NH // CPS + i * _MSL
        zs = [zs_ref[j] for j in range(NZ)]
        for j in range(len(_LP) - 1):
            loop_in(i, j).wait()
        pl.when(i + 1 < _NMID)(lambda: loop_in(i, len(_LP) - 1).wait())

        def guarded(slab, fn):
            pl.when(i >= (hi if slab >= nbl else hi + 1))(fn)

        def after(bi):
            started = False
            if hb <= bi < hb + ng:
                @pl.when(i == hi)
                def _():
                    for rr in bands[(bi - hb) * per:(bi - hb + 1) * per]:
                        out1(0, nb, 0, B, rr, BAND)
                started = True
            if bi == nblk - 2:
                guarded(bi // 2, lambda: out_start(s + bi // 2, T2))
                started = True
            elif bi % 2 == 1 and bi < nblk - 1:
                guarded(bi // 2, lambda: out_start(s + bi // 2, B))
                started = True
            if not started or bi + 1 == nblk:
                return None
            ns, nc = s + (bi + 1) // 2, ((bi + 1) % 2) * T2
            obuf[ns, 0:8, pl.ds(nc, T)] = jnp.zeros((8, T), bf16)
            return pltpu.bitcast(obuf[ns, 0:8, pl.ds(nc, T)].astype(f32)[:, :128], u32)

        def last_done(ss, c0, r0, nr):
            guarded(_MSL - 1, lambda: out1(ss, 1, c0, T2, r0, nr))

        blocks = [(s + bi // 2, (bi % 2) * T2) for bi in range(nblk)]
        return run(blocks, (jnp.minimum(s + _MSL, S - 1), 0), mr, zs, after, last_done)

    lax.fori_loop(0, _NMID, body, mr)
    pltpu.make_async_copy(obuf, o_hbm, osem.at[0]).wait()


@jax.jit
def pallas_standalone__layernorm_linear__sampling_kernel(
    x: jax.Array,
    g: jax.Array,
    b: jax.Array,
    w: jax.Array,
):
    assert x.shape == (B, S, D)
    xt = jnp.transpose(x, (1, 2, 0))
    anyspec = pl.BlockSpec(memory_space=pl.ANY)
    out = pl.pallas_call(
        _kernel,
        in_specs=[anyspec] * 4,
        out_specs=anyspec,
        out_shape=jax.ShapeDtypeStruct((S, D, B), x.dtype),
        scratch_shapes=[
            pltpu.VMEM((S, D, B), bf16), pltpu.VMEM((S, D, B), bf16),
            pltpu.VMEM((D, D), bf16), pltpu.VMEM((D,), bf16), pltpu.VMEM((D,), bf16),
            pltpu.VMEM((49, Q // 2, 128), u32), pltpu.VMEM((D // 2, KR), u32),
            pltpu.VMEM((2, 7, H, T), f32),
            pltpu.VMEM((8, 128), jnp.int32), pltpu.SMEM((NZ,), jnp.int32),
            pltpu.SemaphoreType.DMA((_NSEM_IN,)), pltpu.SemaphoreType.DMA((1,)),
            pltpu.SemaphoreType.DMA((3,)),
        ],
        compiler_params=pltpu.CompilerParams(
            vmem_limit_bytes=110 * 1024 * 1024,
            disable_bounds_checks=True,
            disable_semaphore_checks=True,
        ),
    )(xt, g, b, w)
    return jnp.transpose(out, (2, 0, 1))
```
